```python
import jax
import jax.numpy as jnp

def _softmax(x, axis=-1):
    return jax.nn.softmax(x, axis=axis)
def _gelu(x):
    return jax.nn.gelu(x, approximate=True)
def _silu(x):
    return jax.nn.silu(x)
def _sigmoid(x):
    return jax.nn.sigmoid(x)
def _layernorm(x, axis=-1, eps=1e-5):
    m = jnp.mean(x, axis=axis, keepdims=True)
    v = jnp.var(x, axis=axis, keepdims=True)
    return (x - m) / jnp.sqrt(v + eps)
def _scatter_add(tgt, idx, src, axis=0):
    return tgt.at[idx].add(src)
def _segment_sum(src, seg, n):
    return jax.ops.segment_sum(src, seg, n)
class _Rng:
    def __init__(self, key):
        self._k = key
    def _next(self):
        self._k, sub = jax.random.split(self._k)
        return sub
    def normal(self, shape):
        return jax.random.normal(self._next(), shape, dtype=jnp.bfloat16)
    def randint(self, lo, hi, shape):
        return jax.random.randint(self._next(), shape, lo, hi, dtype=jnp.int32)
    def uniform(self, shape, lo=0.0, hi=1.0):
        return jax.random.uniform(self._next(), shape, jnp.bfloat16, lo, hi)
    def permutation(self, n):
        return jax.random.permutation(self._next(), n)


kernel_name = 'parallel_sum__linear_kernel_hedgehog__glu_gated_bilinear__prompt'

def _fwd_setup_inputs():
    _rng = _Rng(jax.random.key(int.from_bytes(__import__("os").urandom(4), "little")))
    _w = (lambda a: (lambda t: t.astype(jnp.bfloat16) if jnp.issubdtype(t.dtype, jnp.floating) else t)(jnp.asarray(a)))
    def _A_setup():
        B, S, D, H = 1, 2048, 512, 32
        Dh = D // H
        return {
            "x": _w((lambda *s: _rng.normal(s) * 0.05)(B, S, D)),
            "wqkv": _w((lambda *s: _rng.normal(s) * 0.05)(D, 3 * D)),
            "w_phi": _w((lambda *s: _rng.normal(s) * 0.05)(H, Dh, Dh) * (Dh ** -0.5)),
            "wo": _w((lambda *s: _rng.normal(s) * 0.05)(D, D)),
        }
    _A_in = _A_setup()

    def _B_setup():
        B, S, D, F = 1, 2048, 512, 1792
        return {
            "x": _w((lambda *s: _rng.normal(s) * 0.05)(B, S, D)),
            "w_gate": _w((lambda *s: _rng.normal(s) * 0.05)(D, F) * (D ** -0.5)),
            "w_up": _w((lambda *s: _rng.normal(s) * 0.05)(D, F) * (D ** -0.5)),
            "w_down": _w((lambda *s: _rng.normal(s) * 0.05)(F, D) * (F ** -0.5)),
        }
    _B_in = _B_setup()

    return {
        "A_x": _A_in["x"],
        "A_wqkv": _A_in["wqkv"],
        "A_w_phi": _A_in["w_phi"],
        "A_wo": _A_in["wo"],
        "B_x": _B_in["x"],
        "B_w_gate": _B_in["w_gate"],
        "B_w_up": _B_in["w_up"],
        "B_w_down": _B_in["w_down"],
    }

def _fwd_reference(A_x, A_wqkv, A_w_phi, A_wo, B_x, B_w_gate, B_w_up, B_w_down):
    def _A_ref(x, wqkv, w_phi, wo):
        B, S, D = x.shape
        H = 32; Dh = D // H
        qkv = (lambda x, *d: x.transpose(*d))((x @ wqkv).reshape(B, S, 3, H, Dh), 2, 0, 3, 1, 4)
        q, k, v = qkv[0], qkv[1], qkv[2]
        pq = jnp.einsum("bhsd,hdf->bhsf", q, w_phi)
        pk = jnp.einsum("bhsd,hdf->bhsf", k, w_phi)
        phi_q = jnp.concatenate([_softmax(pq, axis=-1), _softmax(-pq, axis=-1)], axis=-1)
        phi_k = jnp.concatenate([_softmax(pk, axis=-1), _softmax(-pk, axis=-1)], axis=-1)
        kv = jnp.einsum("bhsf,bhsd->bhfd", phi_k, v)
        z  = jnp.einsum("bhsf->bhf", phi_k)
        num = jnp.einsum("bhqf,bhfd->bhqd", phi_q, kv)
        den = jnp.einsum("bhqf,bhf->bhq", phi_q, z)[..., None] + 1e-6
        o = num / den
        return (lambda x, *d: x.transpose(*d))(o, 0, 2, 1, 3).reshape(B, S, D) @ wo

    def _B_ref(x, w_gate, w_up, w_down):
        g = jnp.einsum("bsd,df->bsf", x, w_gate)
        u = jnp.einsum("bsd,df->bsf", x, w_up)
        h = g * u
        return jnp.einsum("bsf,fd->bsd", h, w_down)

    x = A_x
    xn = _layernorm(x, axis=-1)
    return x + _A_ref(xn, A_wqkv, A_w_phi, A_wo) + _B_ref(xn, B_w_gate, B_w_up, B_w_down)


def setup_inputs():
    _inp = _fwd_setup_inputs()
    _gk = jax.random.fold_in(jax.random.key(int.from_bytes(__import__("os").urandom(4), "little")), 2**31 - 1)
    _shapes = [[1, 2048, 512]]
    _dtypes = ['bfloat16']
    _gks = jax.random.split(_gk, len(_shapes))
    _gs = [jax.random.normal(k, s, dtype=jnp.dtype(d)) * 0.05 for k, s, d in zip(_gks, _shapes, _dtypes)]
    _inp["grad_out"] = _gs[0]
    return _inp

def reference(A_x, A_wqkv, A_w_phi, A_wo, B_w_gate, B_w_up, B_w_down, B_x, grad_out):
    _const = dict(B_x=B_x)
    def _f(*_d):
        return _fwd_reference(**{'A_x': _d[0], 'A_wqkv': _d[1], 'A_w_phi': _d[2], 'A_wo': _d[3], 'B_w_gate': _d[4], 'B_w_up': _d[5], 'B_w_down': _d[6], **_const})
    _out, _vjp = jax.vjp(_f, A_x, A_wqkv, A_w_phi, A_wo, B_w_gate, B_w_up, B_w_down)
    _grads = _vjp(grad_out)
    _out0 = jnp.asarray(_out)
    return (_out0, *[jnp.asarray(_g) for _g in _grads])
```

```python
import functools
import jax
import jax.numpy as jnp
from jax import lax
import jax.experimental.pallas as pl
import jax.experimental.pallas.tpu as pltpu

S, D, H, DH, F = 2048, 512, 32, 16, 1792
NG = 4
BF = jnp.bfloat16
F32 = jnp.float32

NN = (((1,), (0,)), ((), ()))
NT = (((1,), (1,)), ((), ()))
TN = (((0,), (0,)), ((), ()))


def _dot(a, b, dims=NN):
    return lax.dot_general(a, b, dims, preferred_element_type=F32)


def _iota(shape, dim):
    return lax.broadcasted_iota(jnp.int32, shape, dim)


def _softmax_pair(p):
    T = p.shape[-1]
    p3 = p.reshape(DH, 8, T)
    mx = jnp.max(p3, axis=0, keepdims=True)
    mn = jnp.min(p3, axis=0, keepdims=True)
    ea = jnp.exp(p3 - mx)
    eb = jnp.exp(mn - p3)
    a = ea * (1.0 / jnp.sum(ea, axis=0, keepdims=True))
    b = eb * (1.0 / jnp.sum(eb, axis=0, keepdims=True))
    return a, b


def _softmax_pair_bwd(a, b, da, db):
    dpa = a * (da - jnp.sum(a * da, axis=0, keepdims=True))
    dpb = b * (db - jnp.sum(b * db, axis=0, keepdims=True))
    return dpa - dpb


def _lane_partial(x):
    T = x.shape[-1]
    acc = x[:, 0:128]
    for j in range(1, T // 128):
        acc = acc + x[:, j * 128:(j + 1) * 128]
    return acc


def _layernorm(x):
    m = jnp.mean(x, axis=-1, keepdims=True)
    xc = x - m
    v = jnp.mean(xc * xc, axis=-1, keepdims=True)
    r = lax.rsqrt(v + 1e-5)
    return xc * r, r


def make_kernel(T):
    NTILE = S // T

    def kernel(x_ref, wqkv_ref, wphi_ref, wo_ref, wg_ref, wu_ref, wd_ref, dy_ref,
               out_ref, dx_ref, dwqkv_ref, dwphi_ref, dwo_ref, dwg_ref, dwu_ref, dwd_ref,
               wcat_ref, wqkT_ref, wop_ref, b_ref,
               xn_ref, v_ref, phik_ref, phikb_ref, outp_ref, dxn_ref, dxnT_ref,
               kv_ref, z_ref, dkv_ref, dz_ref,
               kvm_ref, kvmT_ref, zb_ref,
               agw_ref, auw_ref, adwT_ref, gT_ref, awo_ref):
        r128 = _iota((128, 128), 0)
        c128 = _iota((128, 128), 1)
        pm = jnp.where((r128 // 16 == c128 % 8) & (r128 % 16 == c128 // 8), 1.0, 0.0).astype(BF)
        pmT = jnp.where((c128 // 16 == r128 % 8) & (c128 % 16 == r128 // 8), 1.0, 0.0).astype(BF)
        e16 = jnp.where(_iota((16, 128), 1) // 8 == _iota((16, 128), 0), 1.0, 0.0).astype(BF)
        ball = _dot(wphi_ref[...], e16)
        maskb = ((_iota((512, 128), 0) // 16) % 8) == (_iota((512, 128), 1) % 8)
        ball = jnp.where(maskb, ball, 0.0).astype(BF)
        b_ref[...] = ball
        for g in range(NG):
            bg = ball[g * 128:(g + 1) * 128, :]
            for part in range(2):
                w = wqkv_ref[:, part * 512 + g * 128: part * 512 + (g + 1) * 128]
                wp = _dot(w, bg)
                wcat_ref[:, part * 512 + g * 128: part * 512 + (g + 1) * 128] = wp.astype(BF)
                wqkT_ref[part * 512 + g * 128: part * 512 + (g + 1) * 128, :] = wp.T.astype(BF)
            wv = wqkv_ref[:, 1024 + g * 128: 1024 + (g + 1) * 128]
            wcat_ref[:, 1024 + g * 128: 1024 + (g + 1) * 128] = _dot(wv, pm).astype(BF)
            wop_ref[g * 128:(g + 1) * 128, :] = _dot(pmT, wo_ref[g * 128:(g + 1) * 128, :]).astype(BF)

        kv_ref[...] = jnp.zeros_like(kv_ref)
        z_ref[...] = jnp.zeros_like(z_ref)
        dkv_ref[...] = jnp.zeros_like(dkv_ref)
        dz_ref[...] = jnp.zeros_like(dz_ref)
        agw_ref[...] = jnp.zeros_like(agw_ref)
        auw_ref[...] = jnp.zeros_like(auw_ref)
        adwT_ref[...] = jnp.zeros_like(adwT_ref)
        gT_ref[...] = jnp.zeros_like(gT_ref)
        awo_ref[...] = jnp.zeros_like(awo_ref)

        def phase1(i, carry):
            rows = pl.ds(pl.multiple_of(i * T, T), T)
            x = x_ref[rows, :].astype(F32)
            xn, _ = _layernorm(x)
            xnb = xn.astype(BF)
            xn_ref[rows, :] = xnb
            xnT = xn.T.astype(BF)
            dy = dy_ref[rows, :]
            dyT = dy.astype(F32).T.astype(BF)

            pkT = _dot(wqkT_ref[512:1024, :], xnb, NT)
            v = _dot(xnb, wcat_ref[:, 1024:1536]).astype(BF)
            v_ref[rows, :] = v
            for g in range(NG):
                a, b = _softmax_pair(pkT[g * 128:(g + 1) * 128, :])
                phi = jnp.concatenate([a.reshape(128, T), b.reshape(128, T)], axis=0)
                phib = phi.astype(BF)
                phik_ref[i, g * 256:(g + 1) * 256, :] = phi
                phikb_ref[i, g * 256:(g + 1) * 256, :] = phib
                kv_ref[g * 256:(g + 1) * 256, :] += _dot(phib, v[:, g * 128:(g + 1) * 128])
                z_ref[g * 256:(g + 1) * 256, :] += _lane_partial(phi)

            gg = _dot(xnb, wg_ref[...])
            uu = _dot(xnb, wu_ref[...])
            hb = (gg * uu).astype(BF)
            outp_ref[rows, :] = x + _dot(hb, wd_ref[...])
            dh = _dot(dy, wd_ref[...], NT)
            dgb = (dh * uu).astype(BF)
            dub = (dh * gg).astype(BF)
            agw_ref[...] += _dot(xnT, dgb)
            auw_ref[...] += _dot(xnT, dub)
            adwT_ref[...] += _dot(dyT, hb)
            dxn_ref[rows, :] = _dot(dgb, wg_ref[...], NT) + _dot(dub, wu_ref[...], NT)
            return carry

        lax.fori_loop(0, NTILE, phase1, 0)

        dwg_ref[...] = agw_ref[...].astype(BF)
        dwu_ref[...] = auw_ref[...].astype(BF)
        dwd_ref[...] = adwT_ref[...].T.astype(BF)

        maskkv = (_iota((1024, 128), 0) % 8) == (_iota((1024, 128), 1) % 8)
        kvm = jnp.where(maskkv, kv_ref[...], 0.0)
        kvm_ref[...] = kvm.astype(BF)
        for g in range(NG):
            kvmT_ref[g * 128:(g + 1) * 128, :] = kvm[g * 256:(g + 1) * 256, :].T.astype(BF)
        zb_ref[...] = jnp.broadcast_to(jnp.sum(z_ref[...], axis=1, keepdims=True), (1024, 128))

        def phase2(i, carry):
            rows = pl.ds(pl.multiple_of(i * T, T), T)
            xnb = xn_ref[rows, :]
            dy = dy_ref[rows, :]
            pqT = _dot(wqkT_ref[0:512, :], xnb, NT)
            doT = _dot(wop_ref[...], dy, NT)
            o_parts = []
            dp_parts = []
            for g in range(NG):
                a, b = _softmax_pair(pqT[g * 128:(g + 1) * 128, :])
                phi = jnp.concatenate([a.reshape(128, T), b.reshape(128, T)], axis=0)
                phib = phi.astype(BF)
                zg = zb_ref[g * 256:(g + 1) * 256, :]
                zg = jnp.concatenate([zg] * (T // 128), axis=1).reshape(2 * DH, 8, T)
                den = jnp.sum(phi.reshape(2 * DH, 8, T) * zg, axis=0, keepdims=True) + 1e-6
                inv = 1.0 / den
                numT = _dot(kvmT_ref[g * 128:(g + 1) * 128, :], phib)
                oT = numT.reshape(DH, 8, T) * inv
                o_parts.append(oT.reshape(128, T).astype(BF))
                do3 = doT[g * 128:(g + 1) * 128, :].reshape(DH, 8, T)
                dnum = do3 * inv
                dden = -jnp.sum(do3 * oT, axis=0, keepdims=True) * inv
                dnumb = dnum.reshape(128, T).astype(BF)
                dphi = _dot(kvm_ref[g * 256:(g + 1) * 256, :], dnumb).reshape(2 * DH, 8, T) + zg * dden
                dkv_ref[g * 256:(g + 1) * 256, :] += _dot(phib, dnumb, NT)
                dz_ref[g * 256:(g + 1) * 256, :] += _lane_partial(
                    (phi.reshape(2 * DH, 8, T) * dden).reshape(256, T))
                dp = _softmax_pair_bwd(a, b, dphi[0:DH], dphi[DH:2 * DH])
                dp_parts.append(dp.reshape(128, T).astype(BF))
            oT = jnp.concatenate(o_parts, axis=0)
            dpT = jnp.concatenate(dp_parts, axis=0)
            out_ref[rows, :] = (outp_ref[rows, :] + _dot(oT, wop_ref[...], TN)).astype(BF)
            awo_ref[...] += _dot(oT, dy)
            dxnT_ref[i] = _dot(wcat_ref[:, 0:512], dpT)
            gT_ref[0:512, :] += _dot(dpT, xnb)
            return carry

        lax.fori_loop(0, NTILE, phase2, 0)

        dkvm = jnp.where(maskkv, dkv_ref[...], 0.0)
        kvm_ref[...] = dkvm.astype(BF)
        for g in range(NG):
            kvmT_ref[g * 128:(g + 1) * 128, :] = dkvm[g * 256:(g + 1) * 256, :].T.astype(BF)
        zb_ref[...] = jnp.broadcast_to(jnp.sum(dz_ref[...], axis=1, keepdims=True), (1024, 128))
        for g in range(NG):
            dwo_ref[g * 128:(g + 1) * 128, :] = _dot(pm, awo_ref[g * 128:(g + 1) * 128, :].astype(BF)).astype(BF)

        def phase3(i, carry):
            rows = pl.ds(pl.multiple_of(i * T, T), T)
            xnb = xn_ref[rows, :]
            v = v_ref[rows, :]
            dp_parts = []
            dv_parts = []
            for g in range(NG):
                phi = phik_ref[i, g * 256:(g + 1) * 256, :].reshape(2 * DH, 8, T)
                phib = phikb_ref[i, g * 256:(g + 1) * 256, :]
                zg = zb_ref[g * 256:(g + 1) * 256, :]
                zg = jnp.concatenate([zg] * (T // 128), axis=1)
                dphi = (_dot(kvm_ref[g * 256:(g + 1) * 256, :], v[:, g * 128:(g + 1) * 128], NT) + zg
                        ).reshape(2 * DH, 8, T)
                dv_parts.append(_dot(kvmT_ref[g * 128:(g + 1) * 128, :], phib).astype(BF))
                dp = _softmax_pair_bwd(phi[0:DH], phi[DH:2 * DH], dphi[0:DH], dphi[DH:2 * DH])
                dp_parts.append(dp.reshape(128, T).astype(BF))
            dkvT = jnp.concatenate(dp_parts + dv_parts, axis=0)
            dxnT = dxnT_ref[i] + _dot(wcat_ref[:, 512:1536], dkvT)
            gT_ref[512:1536, :] += _dot(dkvT, xnb)
            dxn = dxn_ref[rows, :] + dxnT.T
            x = x_ref[rows, :].astype(F32)
            xn, r = _layernorm(x)
            m1 = jnp.mean(dxn, axis=-1, keepdims=True)
            m2 = jnp.mean(dxn * xn, axis=-1, keepdims=True)
            dx = dy_ref[rows, :].astype(F32) + r * (dxn - m1 - xn * m2)
            dx_ref[rows, :] = dx.astype(BF)
            return carry

        lax.fori_loop(0, NTILE, phase3, 0)

        e16T = jnp.where(_iota((128, 16), 0) // 8 == _iota((128, 16), 1), 1.0, 0.0).astype(BF)
        maskc = (r128 % 8) == (c128 // 16)
        for g in range(NG):
            bg = b_ref[g * 128:(g + 1) * 128, :]
            ct = None
            for part in range(2):
                gt = gT_ref[part * 512 + g * 128: part * 512 + (g + 1) * 128, :].astype(BF)
                dwT = _dot(bg, gt)
                dwqkv_ref[:, part * 512 + g * 128: part * 512 + (g + 1) * 128] = dwT.T.astype(BF)
                c = _dot(gt, wqkv_ref[:, part * 512 + g * 128: part * 512 + (g + 1) * 128])
                ct = c if ct is None else ct + c
            ctm = jnp.where(maskc, ct, 0.0).astype(BF)
            dwphi_ref[g * 128:(g + 1) * 128, :] = _dot(ctm, e16T, TN).astype(BF)
            gv = gT_ref[1024 + g * 128: 1024 + (g + 1) * 128, :].astype(BF)
            dwqkv_ref[:, 1024 + g * 128: 1024 + (g + 1) * 128] = _dot(pm, gv).T.astype(BF)

    scratch = [
        pltpu.VMEM((512, 1536), BF),
        pltpu.VMEM((1024, 512), BF),
        pltpu.VMEM((512, 512), BF),
        pltpu.VMEM((512, 128), BF),
        pltpu.VMEM((S, D), BF),
        pltpu.VMEM((S, D), BF),
        pltpu.VMEM((NTILE, 1024, T), F32),
        pltpu.VMEM((NTILE, 1024, T), BF),
        pltpu.VMEM((S, D), F32),
        pltpu.VMEM((S, D), F32),
        pltpu.VMEM((NTILE, 512, T), F32),
        pltpu.VMEM((1024, 128), F32),
        pltpu.VMEM((1024, 128), F32),
        pltpu.VMEM((1024, 128), F32),
        pltpu.VMEM((1024, 128), F32),
        pltpu.VMEM((1024, 128), BF),
        pltpu.VMEM((512, 256), BF),
        pltpu.VMEM((1024, 128), F32),
        pltpu.VMEM((512, F), F32),
        pltpu.VMEM((512, F), F32),
        pltpu.VMEM((512, F), F32),
        pltpu.VMEM((1536, 512), F32),
        pltpu.VMEM((512, 512), F32),
    ]
    return kernel, scratch


@jax.jit
def pallas_parallel_sum__linear_kernel_hedgehog__glu_gated_bilinear__prompt_kernel(
        A_x, A_wqkv, A_w_phi, A_wo, B_x, B_w_gate, B_w_up, B_w_down, grad_out):
    T = 256
    kernel, scratch = make_kernel(T)
    out_shape = (
        jax.ShapeDtypeStruct((S, D), BF),
        jax.ShapeDtypeStruct((S, D), BF),
        jax.ShapeDtypeStruct((D, 3 * D), BF),
        jax.ShapeDtypeStruct((H * DH, DH), BF),
        jax.ShapeDtypeStruct((D, D), BF),
        jax.ShapeDtypeStruct((D, F), BF),
        jax.ShapeDtypeStruct((D, F), BF),
        jax.ShapeDtypeStruct((F, D), BF),
    )
    outs = pl.pallas_call(
        kernel,
        out_shape=out_shape,
        scratch_shapes=scratch,
        compiler_params=pltpu.CompilerParams(vmem_limit_bytes=120 * 1024 * 1024),
    )(A_x.reshape(S, D), A_wqkv, A_w_phi.reshape(H * DH, DH), A_wo, B_w_gate, B_w_up, B_w_down,
      grad_out.reshape(S, D))
    out, dx, dwqkv, dwphi, dwo, dwg, dwu, dwd = outs
    return (out.reshape(1, S, D), dx.reshape(1, S, D), dwqkv, dwphi.reshape(H, DH, DH), dwo, dwg, dwu, dwd)
```

```python
import contextlib
import jax
import jax.numpy as jnp
from jax import lax
import jax.experimental.pallas as pl
import jax.experimental.pallas.tpu as pltpu

S, D, H, DH, F = 2048, 512, 32, 16, 1792
NG = 4
NQ = 8
BF = jnp.bfloat16
F32 = jnp.float32

NN = (((1,), (0,)), ((), ()))
NT = (((1,), (1,)), ((), ()))
TN = (((0,), (0,)), ((), ()))


def _dot(a, b, dims=NN):
    return lax.dot_general(a, b, dims, preferred_element_type=F32)


def _iota(shape, dim):
    return lax.broadcasted_iota(jnp.int32, shape, dim)


def _sel(cond):
    return jnp.where(cond, 1.0, 0.0).astype(BF)


def _feat(r):
    return ((r % 64) // 8) * 2 + (r % 8) // 4


def _head8(r):
    return ((r % 128) // 64) * 4 + r % 4


def _hred(x, op):
    r = x[0]
    for k in range(1, x.shape[0]):
        r = op(r, x[k])
    r = op(r, pltpu.roll(r, 4, 0))
    return r[None]


def _softmax_pair(p3):
    mx = _hred(p3, jnp.maximum)
    mn = _hred(p3, jnp.minimum)
    ea = jnp.exp(p3 - mx)
    eb = jnp.exp(mn - p3)
    a = ea * (1.0 / _hred(ea, jnp.add))
    b = eb * (1.0 / _hred(eb, jnp.add))
    return a, b


def _softmax_pair_bwd(a, b, da, db):
    dpa = a * (da - _hred(a * da, jnp.add))
    dpb = b * (db - _hred(b * db, jnp.add))
    return dpa - dpb


def _lane_partial(x):
    T = x.shape[-1]
    acc = x[:, 0:128]
    for j in range(1, T // 128):
        acc = acc + x[:, j * 128:(j + 1) * 128]
    return acc


def _layernorm(x):
    m = jnp.mean(x, axis=-1, keepdims=True)
    xc = x - m
    v = jnp.mean(xc * xc, axis=-1, keepdims=True)
    r = lax.rsqrt(v + 1e-5)
    return xc * r, r


def make_kernel(T, scopes):
    NTILE = S // T
    ZR = D // NTILE

    def scope(name):
        return jax.named_scope(name) if scopes else contextlib.nullcontext()

    def kernel(x_hbm, wqkv_hbm, wphi_hbm, wo_hbm, wg_hbm, wu_hbm, wd_hbm, dy_hbm,
               out_hbm, dx_hbm, dwqkv_hbm, dwphi_hbm, dwo_hbm, dwg_hbm, dwu_hbm, dwd_hbm,
               x_ref, wqkv_ref, wphi_ref, wo_ref, wg_ref, wu_ref, wd_ref, dy_ref,
               out_ref, dx_ref, dwqkv_ref, dwphi_ref, dwo_ref, dwg_ref, dwu_ref, dwd_ref,
               sem_x, sem_dy, sem_w, sem_out, sem_dx, sem_dw,
               wcat_ref, wcatT_ref, wop_ref, bT_ref,
               xn_ref, vT_ref, phik_ref, phikb_ref, dxn_ref, dxnT_ref, dkvT_ref,
               kvT_ref, z_ref, dkvTa_ref, dz_ref,
               kvm_ref, kvmT_ref, zb_ref,
               agw_ref, auw_ref, adwT_ref, gT_ref, awo_ref, ct_ref):

        def tile_rows(i):
            if isinstance(i, int):
                return pl.ds(i * T, T)
            return pl.ds(pl.multiple_of(i * T, T), T)

        def cp_x(i):
            return pltpu.make_async_copy(x_hbm.at[tile_rows(i)], x_ref.at[tile_rows(i)], sem_x.at[i])

        def cp_dy(i):
            return pltpu.make_async_copy(dy_hbm.at[tile_rows(i)], dy_ref.at[tile_rows(i)], sem_dy.at[i])

        def cp_out(i):
            return pltpu.make_async_copy(out_ref.at[tile_rows(i)], out_hbm.at[tile_rows(i)], sem_out.at[i])

        def cp_dx(i):
            return pltpu.make_async_copy(dx_ref.at[tile_rows(i)], dx_hbm.at[tile_rows(i)], sem_dx.at[i])

        w_in = [(wphi_hbm, wphi_ref), (wqkv_hbm.at[:, 512:1536], wqkv_ref.at[:, 512:1536]),
                (wqkv_hbm.at[:, 0:512], wqkv_ref.at[:, 0:512]),
                (wg_hbm, wg_ref), (wu_hbm, wu_ref), (wd_hbm, wd_ref), (wo_hbm, wo_ref)]
        cp_w = [pltpu.make_async_copy(s, d, sem_w.at[k]) for k, (s, d) in enumerate(w_in)]
        cp_wphi, cp_wkv, cp_wq, cp_wg, cp_wu, cp_wd, cp_wo = cp_w
        w_out = [(dwg_ref, dwg_hbm), (dwu_ref, dwu_hbm), (dwd_ref, dwd_hbm), (dwo_ref, dwo_hbm),
                 (dwqkv_ref.at[:, 0:512], dwqkv_hbm.at[:, 0:512]),
                 (dwqkv_ref.at[:, 512:1536], dwqkv_hbm.at[:, 512:1536]),
                 (dwphi_ref, dwphi_hbm)]
        cp_o = [pltpu.make_async_copy(s, d, sem_dw.at[k]) for k, (s, d) in enumerate(w_out)]
        cp_dwg, cp_dwu, cp_dwd, cp_dwo, cp_dwq, cp_dwkv, cp_dwphi = cp_o

        def ln_tile(i):
            rows = tile_rows(i)
            xn, _ = _layernorm(x_ref[rows, :].astype(F32))
            xn_ref[rows, :] = xn.astype(BF)

        with scope('setup'):
            cp_wphi.start()
            cp_x(0).start()
            cp_wkv.start()
            cp_x(1).start()

            kvT_ref[...] = jnp.zeros_like(kvT_ref)
            z_ref[...] = jnp.zeros_like(z_ref)
            dkvTa_ref[...] = jnp.zeros_like(dkvTa_ref)
            dz_ref[...] = jnp.zeros_like(dz_ref)

            r128 = _iota((128, 128), 0)
            c128 = _iota((128, 128), 1)
            pm = _sel((r128 // 16 == _head8(c128)) & (r128 % 16 == _feat(c128)))
            pmT = _sel((c128 // 16 == _head8(r128)) & (c128 % 16 == _feat(r128)))
            eh = _sel(_iota((32, 512), 0) == _iota((32, 512), 1) // 16)
            cmask = (_iota((256, 512), 0) // 16) == (_iota((256, 512), 1) % 16)
            rsel = _sel(_iota((128, 256), 1) % 16 == _feat(_iota((128, 256), 0)))
            hmask = _head8(_iota((128, 512), 0)) == ((_iota((128, 512), 1) // 16) % 8)
            cp_wphi.wait()
            w2 = wphi_ref[...].reshape(DH * DH, H)
            y = jnp.where(cmask, _dot(w2, eh), 0.0).astype(BF)
            bT = jnp.where(hmask, _dot(rsel, y), 0.0).astype(BF)
            bT_ref[...] = bT
            cp_x(0).wait()
            ln_tile(0)
            cp_wkv.wait()
            for i in range(2, NTILE):
                cp_x(i).start()
            for g in range(NG):
                bg = bT[:, g * 128:(g + 1) * 128]
                w = wqkv_ref[:, 512 + g * 128: 512 + (g + 1) * 128]
                wcatT_ref[512 + g * 128: 512 + (g + 1) * 128, :] = _dot(bg, w, NT).astype(BF)
                wv = wqkv_ref[:, 1024 + g * 128: 1024 + (g + 1) * 128]
                wcatT_ref[1024 + g * 128: 1024 + (g + 1) * 128, :] = _dot(pmT, wv, NT).astype(BF)

        def phaseA(i, carry):
            rows = tile_rows(i)

            @pl.when(i + 1 < NTILE)
            def _():
                cp_x(i + 1).wait()

            @pl.when(i == 1)
            def _():
                cp_wq.start()
                cp_wo.start()
                cp_wg.start()

            @pl.when(i == 2)
            def _():
                cp_wu.start()
                cp_wd.start()

            @pl.when(i == 4)
            def _():
                for j in range(NTILE):
                    cp_dy(j).start()

            xnb = xn_ref[rows, :]
            ln_tile(jnp.minimum(i + 1, NTILE - 1))
            pvT = _dot(wcatT_ref[512:1536, :], xnb, NT)
            vTb = pvT[512:1024, :].astype(BF)
            vT_ref[i] = vTb
            for q in range(NQ):
                a, b = _softmax_pair(pvT[q * 64:(q + 1) * 64, :].reshape(8, 8, T))
                phi = jnp.concatenate([a.reshape(64, T), b.reshape(64, T)], axis=0)
                phib = phi.astype(BF)
                phik_ref[i, q * 128:(q + 1) * 128, :] = phi
                phikb_ref[i, q * 128:(q + 1) * 128, :] = phib
                kvT_ref[q * 64:(q + 1) * 64, :] += _dot(vTb[q * 64:(q + 1) * 64, :], phib, NT)
                z_ref[q * 128:(q + 1) * 128, :] += _lane_partial(phi)
            return carry

        with scope('phaseA'):
            lax.fori_loop(0, NTILE, phaseA, 0)

        maskkv = (_iota((512, 128), 0) % 4) == (_iota((512, 128), 1) % 4)

        def finish_kv(accT_ref, zacc_ref):
            kvmT = jnp.where(maskkv, accT_ref[...], 0.0)
            kvmT_ref[...] = kvmT.astype(BF)
            for q in range(NQ):
                kvm_ref[q * 128:(q + 1) * 128, :] = kvmT[q * 64:(q + 1) * 64, :].T.astype(BF)
            zb_ref[...] = jnp.broadcast_to(jnp.sum(zacc_ref[...], axis=1, keepdims=True), (1024, 128))

        with scope('midA'):
            cp_wq.wait()
            cp_wo.wait()
            for g in range(NG):
                bg = bT_ref[:, g * 128:(g + 1) * 128]
                w = wqkv_ref[:, g * 128:(g + 1) * 128]
                wcat_ref[:, g * 128:(g + 1) * 128] = _dot(w, bg, NT).astype(BF)
                wcatT_ref[g * 128:(g + 1) * 128, :] = _dot(bg, w, NT).astype(BF)
                wop_ref[g * 128:(g + 1) * 128, :] = _dot(pmT, wo_ref[g * 128:(g + 1) * 128, :]).astype(BF)
            finish_kv(kvT_ref, z_ref)
            cp_wg.wait()
            cp_wu.wait()
            cp_wd.wait()

        def phaseB(i, carry):
            rows = tile_rows(i)
            cp_dy(i).wait()
            xnb = xn_ref[rows, :]
            xnT = xnb.astype(F32).T.astype(BF)
            dy = dy_ref[rows, :]
            dyT = dy.astype(F32).T.astype(BF)
            pqT = _dot(wcatT_ref[0:512, :], xnb, NT)
            doT = _dot(wop_ref[...], dy, NT)
            o_parts = []
            dp_parts = []
            for q in range(NQ):
                a, b = _softmax_pair(pqT[q * 64:(q + 1) * 64, :].reshape(8, 8, T))
                phi = jnp.concatenate([a, b], axis=0)
                phib = phi.reshape(128, T).astype(BF)
                zg = zb_ref[q * 128:(q + 1) * 128, :]
                zg = jnp.concatenate([zg] * (T // 128), axis=1).reshape(16, 8, T)
                den = _hred(phi * zg, jnp.add) + 1e-6
                inv = 1.0 / den
                numT = _dot(kvmT_ref[q * 64:(q + 1) * 64, :], phib)
                oT = numT.reshape(8, 8, T) * inv
                o_parts.append(oT.reshape(64, T).astype(BF))
                do3 = doT[q * 64:(q + 1) * 64, :].reshape(8, 8, T)
                dnum = do3 * inv
                dden = -_hred(do3 * oT, jnp.add) * inv
                dnumb = dnum.reshape(64, T).astype(BF)
                dphi = _dot(kvm_ref[q * 128:(q + 1) * 128, :], dnumb).reshape(16, 8, T) + zg * dden
                dkvTa_ref[q * 64:(q + 1) * 64, :] += _dot(dnumb, phib, NT)
                dz_ref[q * 128:(q + 1) * 128, :] += _lane_partial((phi * dden).reshape(128, T))
                dp = _softmax_pair_bwd(a, b, dphi[0:8], dphi[8:16])
                dp_parts.append(dp.reshape(64, T).astype(BF))
            oT = jnp.concatenate(o_parts, axis=0)
            dpT = jnp.concatenate(dp_parts, axis=0)

            gg = _dot(xnb, wg_ref[...])
            uu = _dot(xnb, wu_ref[...])
            hb = (gg * uu).astype(BF)
            out_ref[rows, :] = (x_ref[rows, :].astype(F32) + _dot(hb, wd_ref[...])
                                + _dot(oT, wop_ref[...], TN)).astype(BF)
            cp_out(i).start()
            dh = _dot(dy, wd_ref[...], NT)
            dgb = (dh * uu).astype(BF)
            dub = (dh * gg).astype(BF)
            nf = i > 0
            agw = jnp.where(nf, agw_ref[...], 0.0) + _dot(xnT, dgb)
            agw_ref[...] = agw
            dwg_ref[...] = agw.astype(BF)
            auw = jnp.where(nf, auw_ref[...], 0.0) + _dot(xnT, dub)
            auw_ref[...] = auw
            dwu_ref[...] = auw.astype(BF)
            adwT = jnp.where(nf, adwT_ref[...], 0.0) + _dot(dyT, hb)
            adwT_ref[...] = adwT
            dwd_ref[...] = adwT.T.astype(BF)
            dxn_ref[rows, :] = _dot(dgb, wg_ref[...], NT) + _dot(dub, wu_ref[...], NT)

            awo_ref[...] = jnp.where(nf, awo_ref[...], 0.0) + _dot(oT, dy)
            dxnT_ref[i] = _dot(wcat_ref[:, 0:512], dpT)
            gT_ref[0:512, :] = jnp.where(nf, gT_ref[0:512, :], 0.0) + _dot(dpT, xnb)
            return carry

        with scope('phaseB'):
            lax.fori_loop(0, NTILE, phaseB, 0)

        def stage1(i):
            rows = tile_rows(i)
            vTb = vT_ref[i]
            dp_parts = []
            dv_parts = []
            for q in range(NQ):
                phi = phik_ref[i, q * 128:(q + 1) * 128, :].reshape(16, 8, T)
                phib = phikb_ref[i, q * 128:(q + 1) * 128, :]
                zg = zb_ref[q * 128:(q + 1) * 128, :]
                zg = jnp.concatenate([zg] * (T // 128), axis=1)
                dphi = (_dot(kvm_ref[q * 128:(q + 1) * 128, :], vTb[q * 64:(q + 1) * 64, :]) + zg
                        ).reshape(16, 8, T)
                dv_parts.append(_dot(kvmT_ref[q * 64:(q + 1) * 64, :], phib).astype(BF))
                dp = _softmax_pair_bwd(phi[0:8], phi[8:16], dphi[0:8], dphi[8:16])
                dp_parts.append(dp.reshape(64, T).astype(BF))
            dkvT = jnp.concatenate(dp_parts + dv_parts, axis=0)
            dkvT_ref[i] = dkvT
            if isinstance(i, int) and i == 0:
                gT_ref[512:1536, :] = _dot(dkvT, xn_ref[rows, :])
            else:
                gT_ref[512:1536, :] += _dot(dkvT, xn_ref[rows, :])

        def stage2(i):
            rows = tile_rows(i)
            dxnT = dxnT_ref[i] + _dot(wcat_ref[:, 512:1536], dkvT_ref[i])
            dxn = dxn_ref[rows, :] + dxnT.T
            x = x_ref[rows, :].astype(F32)
            xn, r = _layernorm(x)
            m1 = jnp.mean(dxn, axis=-1, keepdims=True)
            m2 = jnp.mean(dxn * xn, axis=-1, keepdims=True)
            dx = dy_ref[rows, :].astype(F32) + r * (dxn - m1 - xn * m2)
            dx_ref[rows, :] = dx.astype(BF)
            cp_dx(i).start()

        with scope('midB'):
            cp_dwg.start()
            cp_dwu.start()
            cp_dwd.start()
            finish_kv(dkvTa_ref, dz_ref)
            for g in range(NG):
                bg = bT_ref[:, g * 128:(g + 1) * 128]
                w = wqkv_ref[:, 512 + g * 128: 512 + (g + 1) * 128]
                wcat_ref[:, 512 + g * 128: 512 + (g + 1) * 128] = _dot(w, bg, NT).astype(BF)
                wv = wqkv_ref[:, 1024 + g * 128: 1024 + (g + 1) * 128]
                wcat_ref[:, 1024 + g * 128: 1024 + (g + 1) * 128] = _dot(wv, pm).astype(BF)
            stage1(0)
            for g in range(NG):
                dwo_ref[g * 128:(g + 1) * 128, :] = _dot(pm, awo_ref[g * 128:(g + 1) * 128, :].astype(BF)).astype(BF)
            for g in range(NG):
                bg = bT_ref[:, g * 128:(g + 1) * 128]
                gt = gT_ref[g * 128:(g + 1) * 128, :].astype(BF)
                dwqkv_ref[:, g * 128:(g + 1) * 128] = _dot(gt, bg, TN).astype(BF)
                ct_ref[:, g * 128:(g + 1) * 128] = _dot(gt, wqkv_ref[:, g * 128:(g + 1) * 128])
            cp_dwo.start()
            cp_dwq.start()

        def phaseC(i, carry):
            stage2(i - 1)
            stage1(i)
            return carry

        with scope('phaseC'):
            lax.fori_loop(1, NTILE, phaseC, 0)

        with scope('final'):
            cts = []
            for g in range(NG):
                bg = bT_ref[:, g * 128:(g + 1) * 128]
                gt = gT_ref[512 + g * 128: 512 + (g + 1) * 128, :].astype(BF)
                dwqkv_ref[:, 512 + g * 128: 512 + (g + 1) * 128] = _dot(gt, bg, TN).astype(BF)
                gv = gT_ref[1024 + g * 128: 1024 + (g + 1) * 128, :].astype(BF)
                dwqkv_ref[:, 1024 + g * 128: 1024 + (g + 1) * 128] = _dot(gv, pmT, TN).astype(BF)
                cts.append(ct_ref[:, g * 128:(g + 1) * 128]
                           + _dot(gt, wqkv_ref[:, 512 + g * 128: 512 + (g + 1) * 128]))
            cp_dwkv.start()
            ctm = jnp.where(hmask, jnp.concatenate(cts, axis=1), 0.0).astype(BF)
            zz = jnp.where(cmask, _dot(rsel, ctm, TN), 0.0).astype(BF)
            dwphi_ref[...] = _dot(zz, eh, NT).astype(BF).reshape(DH, DH, H)
            cp_dwphi.start()
            stage2(NTILE - 1)

        with scope('tailwait'):
            for i in range(NTILE):
                cp_out(i).wait()
                cp_dx(i).wait()
            for c in cp_o:
                c.wait()

    scratch = [
        pltpu.VMEM((S, D), BF), pltpu.VMEM((D, 3 * D), BF), pltpu.VMEM((DH, DH, H), BF), pltpu.VMEM((D, D), BF),
        pltpu.VMEM((D, F), BF), pltpu.VMEM((D, F), BF), pltpu.VMEM((F, D), BF), pltpu.VMEM((S, D), BF),
        pltpu.VMEM((S, D), BF), pltpu.VMEM((S, D), BF), pltpu.VMEM((D, 3 * D), BF), pltpu.VMEM((DH, DH, H), BF),
        pltpu.VMEM((D, D), BF), pltpu.VMEM((D, F), BF), pltpu.VMEM((D, F), BF), pltpu.VMEM((F, D), BF),
        pltpu.SemaphoreType.DMA((NTILE,)), pltpu.SemaphoreType.DMA((NTILE,)), pltpu.SemaphoreType.DMA((7,)),
        pltpu.SemaphoreType.DMA((NTILE,)), pltpu.SemaphoreType.DMA((NTILE,)), pltpu.SemaphoreType.DMA((7,)),
        pltpu.VMEM((512, 1536), BF),
        pltpu.VMEM((1536, 512), BF),
        pltpu.VMEM((512, 512), BF),
        pltpu.VMEM((128, 512), BF),
        pltpu.VMEM((S, D), BF),
        pltpu.VMEM((NTILE, 512, T), BF),
        pltpu.VMEM((NTILE, 1024, T), F32),
        pltpu.VMEM((NTILE, 1024, T), BF),
        pltpu.VMEM((S, D), F32),
        pltpu.VMEM((NTILE, 512, T), F32),
        pltpu.VMEM((NTILE, 1024, T), BF),
        pltpu.VMEM((512, 128), F32),
        pltpu.VMEM((1024, 128), F32),
        pltpu.VMEM((512, 128), F32),
        pltpu.VMEM((1024, 128), F32),
        pltpu.VMEM((1024, 64), BF),
        pltpu.VMEM((512, 128), BF),
        pltpu.VMEM((1024, 128), F32),
        pltpu.VMEM((512, F), F32),
        pltpu.VMEM((512, F), F32),
        pltpu.VMEM((512, F), F32),
        pltpu.VMEM((1536, 512), F32),
        pltpu.VMEM((512, 512), F32),
        pltpu.VMEM((128, 512), F32),
    ]
    return kernel, scratch


@jax.jit
def pallas_parallel_sum__linear_kernel_hedgehog__glu_gated_bilinear__prompt_kernel(
        A_x, A_wqkv, A_w_phi, A_wo, B_x, B_w_gate, B_w_up, B_w_down, grad_out):
    T, scopes = 256, 0
    kernel, scratch = make_kernel(T, scopes)
    out_shape = (
        jax.ShapeDtypeStruct((S, D), BF),
        jax.ShapeDtypeStruct((S, D), BF),
        jax.ShapeDtypeStruct((D, 3 * D), BF),
        jax.ShapeDtypeStruct((DH, DH, H), BF),
        jax.ShapeDtypeStruct((D, D), BF),
        jax.ShapeDtypeStruct((D, F), BF),
        jax.ShapeDtypeStruct((D, F), BF),
        jax.ShapeDtypeStruct((F, D), BF),
    )
    anyspec = pl.BlockSpec(memory_space=pl.ANY)
    outs = pl.pallas_call(
        kernel,
        out_shape=out_shape,
        in_specs=[anyspec] * 8,
        out_specs=[anyspec] * 8,
        scratch_shapes=scratch,
        compiler_params=pltpu.CompilerParams(vmem_limit_bytes=120 * 1024 * 1024),
    )(A_x.reshape(S, D), A_wqkv, jnp.transpose(A_w_phi, (1, 2, 0)), A_wo, B_w_gate, B_w_up, B_w_down,
      grad_out.reshape(S, D))
    out, dx, dwqkv, dwphi, dwo, dwg, dwu, dwd = outs
    return (out.reshape(1, S, D), dx.reshape(1, S, D), dwqkv, jnp.transpose(dwphi, (2, 0, 1)), dwo, dwg, dwu, dwd)
```

```python
import contextlib
import jax
import jax.numpy as jnp
from jax import lax
import jax.experimental.pallas as pl
import jax.experimental.pallas.tpu as pltpu

S, D, H, DH, F = 2048, 512, 32, 16, 1792
NG = 4
NQ = 8
BF = jnp.bfloat16
F32 = jnp.float32

NN = (((1,), (0,)), ((), ()))
NT = (((1,), (1,)), ((), ()))
TN = (((0,), (0,)), ((), ()))


def _dot(a, b, dims=NN):
    return lax.dot_general(a, b, dims, preferred_element_type=F32)


def _iota(shape, dim):
    return lax.broadcasted_iota(jnp.int32, shape, dim)


def _sel(cond):
    return jnp.where(cond, 1.0, 0.0).astype(BF)


def _feat(r):
    return ((r % 64) // 8) * 2 + (r % 8) // 4


def _head8(r):
    return ((r % 128) // 64) * 4 + r % 4


def _hred(x, op):
    r = x[0]
    for k in range(1, x.shape[0]):
        r = op(r, x[k])
    r = op(r, pltpu.roll(r, 4, 0))
    return r[None]


def _softmax_pair(p3):
    mx = _hred(p3, jnp.maximum)
    mn = _hred(p3, jnp.minimum)
    ea = jnp.exp(p3 - mx)
    eb = jnp.exp(mn - p3)
    a = ea * (1.0 / _hred(ea, jnp.add))
    b = eb * (1.0 / _hred(eb, jnp.add))
    return a, b


def _softmax_pair_bwd(a, b, da, db):
    dpa = a * (da - _hred(a * da, jnp.add))
    dpb = b * (db - _hred(b * db, jnp.add))
    return dpa - dpb


def _lane_partial(x):
    T = x.shape[-1]
    acc = x[:, 0:128]
    for j in range(1, T // 128):
        acc = acc + x[:, j * 128:(j + 1) * 128]
    return acc


def _layernorm(x):
    m = jnp.mean(x, axis=-1, keepdims=True)
    xc = x - m
    v = jnp.mean(xc * xc, axis=-1, keepdims=True)
    r = lax.rsqrt(v + 1e-5)
    return xc * r, r


def make_kernel(T, scopes):
    NTILE = S // T
    ZR = D // NTILE

    def scope(name):
        return jax.named_scope(name) if scopes else contextlib.nullcontext()

    def kernel(x_hbm, wqkv_hbm, wphi_hbm, wo_hbm, wg_hbm, wu_hbm, wd_hbm, dy_hbm,
               out_hbm, dx_hbm, dwqkv_hbm, dwphi_hbm, dwo_hbm, dwg_hbm, dwu_hbm, dwd_hbm,
               x_ref, wqkv_ref, wphi_ref, wo_ref, wg_ref, wu_ref, wd_ref, dy_ref,
               out_ref, dx_ref, dwqkv_ref, dwphi_ref, dwo_ref, dwg_ref, dwu_ref, dwd_ref,
               sem_x, sem_dy, sem_w, sem_out, sem_dx, sem_dw,
               wcat_ref, wcatT_ref, wop_ref, bT_ref,
               xn_ref, vT_ref, phik_ref, phikb_ref, dxn_ref, dxnT_ref, dkvT_ref,
               kvT_ref, z_ref, dkvTa_ref, dz_ref,
               kvm_ref, kvmT_ref, zb_ref,
               agw_ref, auw_ref, adwT_ref, gT_ref, awo_ref, ct_ref):

        def tile_rows(i):
            if isinstance(i, int):
                return pl.ds(i * T, T)
            return pl.ds(pl.multiple_of(i * T, T), T)

        def cp_x(i):
            return pltpu.make_async_copy(x_hbm.at[tile_rows(i)], x_ref.at[tile_rows(i)], sem_x.at[i])

        def cp_dy(i):
            return pltpu.make_async_copy(dy_hbm.at[tile_rows(i)], dy_ref.at[tile_rows(i)], sem_dy.at[i])

        def cp_out(i):
            return pltpu.make_async_copy(out_ref.at[tile_rows(i)], out_hbm.at[tile_rows(i)], sem_out.at[0])

        def cp_dx(i):
            return pltpu.make_async_copy(dx_ref.at[tile_rows(i)], dx_hbm.at[tile_rows(i)], sem_dx.at[0])

        w_in = [(wphi_hbm, wphi_ref), (wqkv_hbm.at[:, 512:1024], wqkv_ref.at[:, 512:1024]),
                (wqkv_hbm.at[:, 0:512], wqkv_ref.at[:, 0:512]),
                (wg_hbm, wg_ref), (wu_hbm, wu_ref), (wd_hbm, wd_ref), (wo_hbm, wo_ref),
                (wqkv_hbm.at[:, 1024:1536], wqkv_ref.at[:, 1024:1536])]
        cp_w = [pltpu.make_async_copy(s, d, sem_w.at[k]) for k, (s, d) in enumerate(w_in)]
        cp_wphi, cp_wk, cp_wq, cp_wg, cp_wu, cp_wd, cp_wo, cp_wv = cp_w
        w_out = [(dwg_ref, dwg_hbm), (dwu_ref, dwu_hbm), (dwd_ref, dwd_hbm), (dwo_ref, dwo_hbm),
                 (dwqkv_ref.at[:, 0:512], dwqkv_hbm.at[:, 0:512]),
                 (dwqkv_ref.at[:, 512:1536], dwqkv_hbm.at[:, 512:1536]),
                 (dwphi_ref, dwphi_hbm)]
        cp_o = [pltpu.make_async_copy(s, d, sem_dw.at[k]) for k, (s, d) in enumerate(w_out)]
        cp_dwg, cp_dwu, cp_dwd, cp_dwo, cp_dwq, cp_dwkv, cp_dwphi = cp_o

        def ln_tile(i):
            rows = tile_rows(i)
            xn, _ = _layernorm(x_ref[rows, :].astype(F32))
            xn_ref[rows, :] = xn.astype(BF)

        with scope('setup'):
            cp_wphi.start()
            cp_wk.start()
            cp_x(0).start()
            cp_wv.start()


            r128 = _iota((128, 128), 0)
            c128 = _iota((128, 128), 1)
            pm = _sel((r128 // 16 == _head8(c128)) & (r128 % 16 == _feat(c128)))
            pmT = _sel((c128 // 16 == _head8(r128)) & (c128 % 16 == _feat(r128)))
            eh = _sel(_iota((32, 512), 0) == _iota((32, 512), 1) // 16)
            cmask = (_iota((256, 512), 0) // 16) == (_iota((256, 512), 1) % 16)
            rsel = _sel(_iota((128, 256), 1) % 16 == _feat(_iota((128, 256), 0)))
            hmask = _head8(_iota((128, 512), 0)) == ((_iota((128, 512), 1) // 16) % 8)
            cp_wphi.wait()
            w2 = wphi_ref[...].reshape(DH * DH, H)
            y = jnp.where(cmask, _dot(w2, eh), 0.0).astype(BF)
            bT = jnp.where(hmask, _dot(rsel, y), 0.0).astype(BF)
            bT_ref[...] = bT
            cp_x(0).wait()
            cp_wk.wait()
            cp_x(1).start()
            ln_tile(0)
            for g in range(NG):
                bg = bT[:, g * 128:(g + 1) * 128]
                w = wqkv_ref[:, 512 + g * 128: 512 + (g + 1) * 128]
                wcatT_ref[512 + g * 128: 512 + (g + 1) * 128, :] = _dot(bg, w, NT).astype(BF)
            cp_wv.wait()
            for i in range(2, NTILE):
                cp_x(i).start()
            for g in range(NG):
                wv = wqkv_ref[:, 1024 + g * 128: 1024 + (g + 1) * 128]
                wcatT_ref[1024 + g * 128: 1024 + (g + 1) * 128, :] = _dot(pmT, wv, NT).astype(BF)

        def phaseA(i, carry):
            rows = tile_rows(i)

            @pl.when(i + 1 < NTILE)
            def _():
                cp_x(i + 1).wait()

            @pl.when(i == 1)
            def _():
                cp_wq.start()
                cp_wo.start()
                cp_wg.start()

            @pl.when(i == 2)
            def _():
                cp_wu.start()
                cp_wd.start()

            @pl.when(i == 4)
            def _():
                for j in range(NTILE):
                    cp_dy(j).start()

            xnb = xn_ref[rows, :]
            ln_tile(jnp.minimum(i + 1, NTILE - 1))
            pvT = _dot(wcatT_ref[512:1536, :], xnb, NT)
            vTb = pvT[512:1024, :].astype(BF)
            vT_ref[i] = vTb
            ones16 = jnp.ones((16, T), BF)
            for q in range(NQ):
                a, b = _softmax_pair(pvT[q * 64:(q + 1) * 64, :].reshape(8, 8, T))
                phi = jnp.concatenate([a.reshape(64, T), b.reshape(64, T)], axis=0)
                phib = phi.astype(BF)
                phik_ref[i, q * 128:(q + 1) * 128, :] = phi
                phikb_ref[i, q * 128:(q + 1) * 128, :] = phib
                vq = jnp.concatenate([vTb[q * 64:(q + 1) * 64, :], ones16], axis=0)
                kz = _dot(vq, phib, NT)
                kvT_ref[q * 64:(q + 1) * 64, :] = jnp.where(i > 0, kvT_ref[q * 64:(q + 1) * 64, :], 0.0) + kz[0:64]
                z_ref[q * 8:(q + 1) * 8, :] = jnp.where(i > 0, z_ref[q * 8:(q + 1) * 8, :], 0.0) + kz[64:72]
            return carry

        with scope('phaseA'):
            lax.fori_loop(0, NTILE, phaseA, 0)

        maskkv = (_iota((512, 128), 0) % 4) == (_iota((512, 128), 1) % 4)

        def finish_kv(accT_ref, zacc_ref, rowform):
            kvmT = jnp.where(maskkv, accT_ref[...], 0.0)
            kvmT_ref[...] = kvmT.astype(BF)
            for q in range(NQ):
                kvm_ref[q * 128:(q + 1) * 128, :] = kvmT[q * 64:(q + 1) * 64, :].T.astype(BF)
            if rowform:
                for q in range(NQ):
                    zrow = zacc_ref[q * 8:q * 8 + 1, :]
                    zb_ref[q * 128:(q + 1) * 128, :] = jnp.broadcast_to(zrow, (128, 128)).T
            else:
                zb_ref[...] = jnp.broadcast_to(jnp.sum(zacc_ref[...], axis=1, keepdims=True), (1024, 128))

        with scope('midA'):
            cp_wq.wait()
            cp_wo.wait()
            for g in range(NG):
                bg = bT_ref[:, g * 128:(g + 1) * 128]
                w = wqkv_ref[:, g * 128:(g + 1) * 128]
                wpT = _dot(bg, w, NT)
                wcat_ref[:, g * 128:(g + 1) * 128] = wpT.T.astype(BF)
                wcatT_ref[g * 128:(g + 1) * 128, :] = wpT.astype(BF)
                wop_ref[g * 128:(g + 1) * 128, :] = _dot(pmT, wo_ref[g * 128:(g + 1) * 128, :]).astype(BF)
            finish_kv(kvT_ref, z_ref, True)
            cp_wg.wait()
            cp_wu.wait()
            cp_wd.wait()

        def phaseB(i, carry):
            rows = tile_rows(i)
            cp_dy(i).wait()
            xnb = xn_ref[rows, :]
            xnT = xnb.astype(F32).T.astype(BF)
            dy = dy_ref[rows, :]
            dyT = dy.astype(F32).T.astype(BF)
            pqT = _dot(wcatT_ref[0:512, :], xnb, NT)
            doT = _dot(wop_ref[...], dy, NT)
            o_parts = []
            dp_parts = []
            g_parts = []
            u_parts = []
            for q in range(NQ):
                a, b = _softmax_pair(pqT[q * 64:(q + 1) * 64, :].reshape(8, 8, T))
                phi = jnp.concatenate([a, b], axis=0)
                phib = phi.reshape(128, T).astype(BF)
                zg = zb_ref[q * 128:(q + 1) * 128, :]
                zg = jnp.concatenate([zg] * (T // 128), axis=1).reshape(16, 8, T)
                den = _hred(phi * zg, jnp.add) + 1e-6
                inv = 1.0 / den
                numT = _dot(kvmT_ref[q * 64:(q + 1) * 64, :], phib)
                oT = numT.reshape(8, 8, T) * inv
                o_parts.append(oT.reshape(64, T).astype(BF))
                do3 = doT[q * 64:(q + 1) * 64, :].reshape(8, 8, T)
                dnum = do3 * inv
                dden = -_hred(do3 * oT, jnp.add) * inv
                dnumb = dnum.reshape(64, T).astype(BF)
                dphi = _dot(kvm_ref[q * 128:(q + 1) * 128, :], dnumb).reshape(16, 8, T) + zg * dden
                dkvTa_ref[q * 64:(q + 1) * 64, :] = (
                    jnp.where(i > 0, dkvTa_ref[q * 64:(q + 1) * 64, :], 0.0) + _dot(dnumb, phib, NT))
                dz_ref[q * 128:(q + 1) * 128, :] = (
                    jnp.where(i > 0, dz_ref[q * 128:(q + 1) * 128, :], 0.0)
                    + _lane_partial((phi * dden).reshape(128, T)))
                dp = _softmax_pair_bwd(a, b, dphi[0:8], dphi[8:16])
                dp_parts.append(dp.reshape(64, T).astype(BF))
                if q < 7:
                    g_parts.append(_dot(xnb, wg_ref[:, q * 256:(q + 1) * 256]))
                    u_parts.append(_dot(xnb, wu_ref[:, q * 256:(q + 1) * 256]))
            oT = jnp.concatenate(o_parts, axis=0)
            dpT = jnp.concatenate(dp_parts, axis=0)

            gg = jnp.concatenate(g_parts, axis=1)
            uu = jnp.concatenate(u_parts, axis=1)
            hb = (gg * uu).astype(BF)
            out_ref[rows, :] = (x_ref[rows, :].astype(F32) + _dot(hb, wd_ref[...])
                                + _dot(oT, wop_ref[...], TN)).astype(BF)
            cp_out(i).start()
            dh = _dot(dy, wd_ref[...], NT)
            dgb = (dh * uu).astype(BF)
            dub = (dh * gg).astype(BF)
            nf = i > 0
            agw = jnp.where(nf, agw_ref[...], 0.0) + _dot(xnT, dgb)
            agw_ref[...] = agw
            dwg_ref[...] = agw.astype(BF)
            auw = jnp.where(nf, auw_ref[...], 0.0) + _dot(xnT, dub)
            auw_ref[...] = auw
            dwu_ref[...] = auw.astype(BF)
            adwT = jnp.where(nf, adwT_ref[...], 0.0) + _dot(dyT, hb)
            adwT_ref[...] = adwT
            dwd_ref[...] = adwT.T.astype(BF)
            dxn_ref[rows, :] = _dot(dgb, wg_ref[...], NT) + _dot(dub, wu_ref[...], NT)

            awo_ref[...] = jnp.where(nf, awo_ref[...], 0.0) + _dot(oT, dy)
            dxnT_ref[i] = _dot(wcat_ref[:, 0:512], dpT)
            gT_ref[0:512, :] = jnp.where(nf, gT_ref[0:512, :], 0.0) + _dot(dpT, xnb)
            return carry

        with scope('phaseB'):
            lax.fori_loop(0, NTILE, phaseB, 0)

        def stage1(i):
            rows = tile_rows(i)
            vTb = vT_ref[i]
            dp_parts = []
            dv_parts = []
            for q in range(NQ):
                phi = phik_ref[i, q * 128:(q + 1) * 128, :].reshape(16, 8, T)
                phib = phikb_ref[i, q * 128:(q + 1) * 128, :]
                zg = zb_ref[q * 128:(q + 1) * 128, :]
                zg = jnp.concatenate([zg] * (T // 128), axis=1)
                dphi = (_dot(kvm_ref[q * 128:(q + 1) * 128, :], vTb[q * 64:(q + 1) * 64, :]) + zg
                        ).reshape(16, 8, T)
                dv_parts.append(_dot(kvmT_ref[q * 64:(q + 1) * 64, :], phib).astype(BF))
                dp = _softmax_pair_bwd(phi[0:8], phi[8:16], dphi[0:8], dphi[8:16])
                dp_parts.append(dp.reshape(64, T).astype(BF))
            dkvT = jnp.concatenate(dp_parts + dv_parts, axis=0)
            dkvT_ref[i] = dkvT
            if isinstance(i, int) and i == 0:
                gT_ref[512:1536, :] = _dot(dkvT, xn_ref[rows, :])
            else:
                gT_ref[512:1536, :] += _dot(dkvT, xn_ref[rows, :])

        def stage2(i):
            rows = tile_rows(i)
            dxnT = dxnT_ref[i] + _dot(wcat_ref[:, 512:1536], dkvT_ref[i])
            dxn = dxn_ref[rows, :] + dxnT.T
            x = x_ref[rows, :].astype(F32)
            xn, r = _layernorm(x)
            m1 = jnp.mean(dxn, axis=-1, keepdims=True)
            m2 = jnp.mean(dxn * xn, axis=-1, keepdims=True)
            dx = dy_ref[rows, :].astype(F32) + r * (dxn - m1 - xn * m2)
            dx_ref[rows, :] = dx.astype(BF)
            cp_dx(i).start()

        with scope('midB'):
            cp_dwg.start()
            cp_dwu.start()
            cp_dwd.start()
            finish_kv(dkvTa_ref, dz_ref, False)
            wcat_ref[:, 512:1536] = wcatT_ref[512:1536, :].astype(F32).T.astype(BF)
            stage1(0)
            for g in range(NG):
                dwo_ref[g * 128:(g + 1) * 128, :] = _dot(pm, awo_ref[g * 128:(g + 1) * 128, :].astype(BF)).astype(BF)
            for g in range(NG):
                bg = bT_ref[:, g * 128:(g + 1) * 128]
                gt = gT_ref[g * 128:(g + 1) * 128, :].astype(BF)
                dwqkv_ref[:, g * 128:(g + 1) * 128] = _dot(gt, bg, TN).astype(BF)
                ct_ref[:, g * 128:(g + 1) * 128] = _dot(gt, wqkv_ref[:, g * 128:(g + 1) * 128])
            cp_dwo.start()
            cp_dwq.start()

        def phaseC(i, carry):
            stage2(i - 1)
            stage1(i)
            return carry

        with scope('phaseC'):
            lax.fori_loop(1, NTILE, phaseC, 0)

        with scope('final'):
            gts = []
            for g in range(NG):
                bg = bT_ref[:, g * 128:(g + 1) * 128]
                gt = gT_ref[512 + g * 128: 512 + (g + 1) * 128, :].astype(BF)
                gts.append(gt)
                dwqkv_ref[:, 512 + g * 128: 512 + (g + 1) * 128] = _dot(gt, bg, TN).astype(BF)
                gv = gT_ref[1024 + g * 128: 1024 + (g + 1) * 128, :].astype(BF)
                dwqkv_ref[:, 1024 + g * 128: 1024 + (g + 1) * 128] = _dot(gv, pmT, TN).astype(BF)
            cp_dwkv.start()
            stage2(NTILE - 1)
            cts = []
            for g in range(NG):
                cts.append(ct_ref[:, g * 128:(g + 1) * 128]
                           + _dot(gts[g], wqkv_ref[:, 512 + g * 128: 512 + (g + 1) * 128]))
            ctm = jnp.where(hmask, jnp.concatenate(cts, axis=1), 0.0).astype(BF)
            zz = jnp.where(cmask, _dot(rsel, ctm, TN), 0.0).astype(BF)
            dwphi_ref[...] = _dot(zz, eh, NT).astype(BF).reshape(DH, DH, H)
            cp_dwphi.start()

        with scope('tailwait'):
            pltpu.make_async_copy(out_ref, out_hbm, sem_out.at[0]).wait()
            for c in cp_o:
                c.wait()
            pltpu.make_async_copy(dx_ref, dx_hbm, sem_dx.at[0]).wait()

    scratch = [
        pltpu.VMEM((S, D), BF), pltpu.VMEM((D, 3 * D), BF), pltpu.VMEM((DH, DH, H), BF), pltpu.VMEM((D, D), BF),
        pltpu.VMEM((D, F), BF), pltpu.VMEM((D, F), BF), pltpu.VMEM((F, D), BF), pltpu.VMEM((S, D), BF),
        pltpu.VMEM((S, D), BF), pltpu.VMEM((S, D), BF), pltpu.VMEM((D, 3 * D), BF), pltpu.VMEM((DH, DH, H), BF),
        pltpu.VMEM((D, D), BF), pltpu.VMEM((D, F), BF), pltpu.VMEM((D, F), BF), pltpu.VMEM((F, D), BF),
        pltpu.SemaphoreType.DMA((NTILE,)), pltpu.SemaphoreType.DMA((NTILE,)), pltpu.SemaphoreType.DMA((8,)),
        pltpu.SemaphoreType.DMA((NTILE,)), pltpu.SemaphoreType.DMA((NTILE,)), pltpu.SemaphoreType.DMA((7,)),
        pltpu.VMEM((512, 1536), BF),
        pltpu.VMEM((1536, 512), BF),
        pltpu.VMEM((512, 512), BF),
        pltpu.VMEM((128, 512), BF),
        pltpu.VMEM((S, D), BF),
        pltpu.VMEM((NTILE, 512, T), BF),
        pltpu.VMEM((NTILE, 1024, T), F32),
        pltpu.VMEM((NTILE, 1024, T), BF),
        pltpu.VMEM((S, D), F32),
        pltpu.VMEM((NTILE, 512, T), F32),
        pltpu.VMEM((NTILE, 1024, T), BF),
        pltpu.VMEM((512, 128), F32),
        pltpu.VMEM((64, 128), F32),
        pltpu.VMEM((512, 128), F32),
        pltpu.VMEM((1024, 128), F32),
        pltpu.VMEM((1024, 64), BF),
        pltpu.VMEM((512, 128), BF),
        pltpu.VMEM((1024, 128), F32),
        pltpu.VMEM((512, F), F32),
        pltpu.VMEM((512, F), F32),
        pltpu.VMEM((512, F), F32),
        pltpu.VMEM((1536, 512), F32),
        pltpu.VMEM((512, 512), F32),
        pltpu.VMEM((128, 512), F32),
    ]
    return kernel, scratch


@jax.jit
def pallas_parallel_sum__linear_kernel_hedgehog__glu_gated_bilinear__prompt_kernel(
        A_x, A_wqkv, A_w_phi, A_wo, B_x, B_w_gate, B_w_up, B_w_down, grad_out):
    T, scopes = 256, 0
    kernel, scratch = make_kernel(T, scopes)
    out_shape = (
        jax.ShapeDtypeStruct((S, D), BF),
        jax.ShapeDtypeStruct((S, D), BF),
        jax.ShapeDtypeStruct((D, 3 * D), BF),
        jax.ShapeDtypeStruct((DH, DH, H), BF),
        jax.ShapeDtypeStruct((D, D), BF),
        jax.ShapeDtypeStruct((D, F), BF),
        jax.ShapeDtypeStruct((D, F), BF),
        jax.ShapeDtypeStruct((F, D), BF),
    )
    anyspec = pl.BlockSpec(memory_space=pl.ANY)
    outs = pl.pallas_call(
        kernel,
        out_shape=out_shape,
        in_specs=[anyspec] * 8,
        out_specs=[anyspec] * 8,
        scratch_shapes=scratch,
        compiler_params=pltpu.CompilerParams(vmem_limit_bytes=120 * 1024 * 1024),
    )(A_x.reshape(S, D), A_wqkv, jnp.transpose(A_w_phi, (1, 2, 0)), A_wo, B_w_gate, B_w_up, B_w_down,
      grad_out.reshape(S, D))
    out, dx, dwqkv, dwphi, dwo, dwg, dwu, dwd = outs
    return (out.reshape(1, S, D), dx.reshape(1, S, D), dwqkv, jnp.transpose(dwphi, (2, 0, 1)), dwo, dwg, dwu, dwd)
```

```python
import jax
import jax.numpy as jnp
from jax import lax
import jax.experimental.pallas as pl
import jax.experimental.pallas.tpu as pltpu

S, D, H, DH, F = 2048, 512, 32, 16, 1792
NG = 4
NQ = 8
BF = jnp.bfloat16
F32 = jnp.float32

NN = (((1,), (0,)), ((), ()))
NT = (((1,), (1,)), ((), ()))
TN = (((0,), (0,)), ((), ()))


def _dot(a, b, dims=NN):
    return lax.dot_general(a, b, dims, preferred_element_type=F32)


def _iota(shape, dim):
    return lax.broadcasted_iota(jnp.int32, shape, dim)


def _sel(cond):
    return jnp.where(cond, 1.0, 0.0).astype(BF)


def _feat(r):
    return ((r % 64) // 8) * 2 + (r % 8) // 4


def _head8(r):
    return ((r % 128) // 64) * 4 + r % 4


def _hred(x, op):
    r = x[0]
    for k in range(1, x.shape[0]):
        r = op(r, x[k])
    r = op(r, pltpu.roll(r, 4, 0))
    return r[None]


def _softmax_pair(p3):
    mx = _hred(p3, jnp.maximum)
    mn = _hred(p3, jnp.minimum)
    ea = jnp.exp(p3 - mx)
    eb = jnp.exp(mn - p3)
    a = ea * (1.0 / _hred(ea, jnp.add))
    b = eb * (1.0 / _hred(eb, jnp.add))
    return a, b


def _softmax_pair_bwd(a, b, da, db):
    dpa = a * (da - _hred(a * da, jnp.add))
    dpb = b * (db - _hred(b * db, jnp.add))
    return dpa - dpb


def _lane_partial(x):
    T = x.shape[-1]
    acc = x[:, 0:128]
    for j in range(1, T // 128):
        acc = acc + x[:, j * 128:(j + 1) * 128]
    return acc


def _layernorm(x):
    m = jnp.mean(x, axis=-1, keepdims=True)
    xc = x - m
    v = jnp.mean(xc * xc, axis=-1, keepdims=True)
    r = lax.rsqrt(v + 1e-5)
    return xc * r, r


def _make_kernel(T):
    NTILE = S // T

    def kernel(x_hbm, wqkv_hbm, wphi_hbm, wo_hbm, wg_hbm, wu_hbm, wd_hbm, dy_hbm,
               out_hbm, dx_hbm, dwqkv_hbm, dwphi_hbm, dwo_hbm, dwg_hbm, dwu_hbm, dwd_hbm,
               x_ref, wqkv_ref, wphi_ref, wo_ref, wg_ref, wu_ref, wd_ref, dy_ref,
               out_ref, dx_ref, dwqkv_ref, dwphi_ref, dwo_ref, dwg_ref, dwu_ref, dwd_ref,
               sem_x, sem_dy, sem_w, sem_out, sem_dx, sem_dw,
               wcat_ref, wcatT_ref, wop_ref, bT_ref,
               xn_ref, vT_ref, phik_ref, phikb_ref, dxn_ref, dxnT_ref, dkvT_ref,
               kvT_ref, z_ref, dkvTa_ref, dz_ref,
               kvm_ref, kvmT_ref, zb_ref,
               agw_ref, auw_ref, adwT_ref, gT_ref, awo_ref, ct_ref):

        def tile_rows(i):
            if isinstance(i, int):
                return pl.ds(i * T, T)
            return pl.ds(pl.multiple_of(i * T, T), T)

        def cp_x(i):
            return pltpu.make_async_copy(x_hbm.at[tile_rows(i)], x_ref.at[tile_rows(i)], sem_x.at[i])

        def cp_dy(i):
            return pltpu.make_async_copy(dy_hbm.at[tile_rows(i)], dy_ref.at[tile_rows(i)], sem_dy.at[i])

        def cp_out(i):
            return pltpu.make_async_copy(out_ref.at[tile_rows(i)], out_hbm.at[tile_rows(i)], sem_out.at[0])

        def cp_dx(i):
            return pltpu.make_async_copy(dx_ref.at[tile_rows(i)], dx_hbm.at[tile_rows(i)], sem_dx.at[0])

        w_in = [(wphi_hbm, wphi_ref), (wqkv_hbm.at[:, 512:1024], wqkv_ref.at[:, 512:1024]),
                (wqkv_hbm.at[:, 0:512], wqkv_ref.at[:, 0:512]),
                (wg_hbm, wg_ref), (wu_hbm, wu_ref), (wd_hbm, wd_ref), (wo_hbm, wo_ref),
                (wqkv_hbm.at[:, 1024:1536], wqkv_ref.at[:, 1024:1536])]
        cp_w = [pltpu.make_async_copy(s, d, sem_w.at[k]) for k, (s, d) in enumerate(w_in)]
        cp_wphi, cp_wk, cp_wq, cp_wg, cp_wu, cp_wd, cp_wo, cp_wv = cp_w
        w_out = [(dwg_ref, dwg_hbm), (dwu_ref, dwu_hbm), (dwd_ref, dwd_hbm), (dwo_ref, dwo_hbm),
                 (dwqkv_ref.at[:, 0:512], dwqkv_hbm.at[:, 0:512]),
                 (dwqkv_ref.at[:, 512:1536], dwqkv_hbm.at[:, 512:1536]),
                 (dwphi_ref, dwphi_hbm)]
        cp_o = [pltpu.make_async_copy(s, d, sem_dw.at[k]) for k, (s, d) in enumerate(w_out)]
        cp_dwg, cp_dwu, cp_dwd, cp_dwo, cp_dwq, cp_dwkv, cp_dwphi = cp_o

        def ln_tile(i):
            rows = tile_rows(i)
            xn, _ = _layernorm(x_ref[rows, :].astype(F32))
            xn_ref[rows, :] = xn.astype(BF)

        cp_wphi.start()
        cp_wk.start()
        cp_x(0).start()
        cp_wv.start()

        r128 = _iota((128, 128), 0)
        c128 = _iota((128, 128), 1)
        pm = _sel((r128 // 16 == _head8(c128)) & (r128 % 16 == _feat(c128)))
        pmT = _sel((c128 // 16 == _head8(r128)) & (c128 % 16 == _feat(r128)))
        eh = _sel(_iota((32, 512), 0) == _iota((32, 512), 1) // 16)
        cmask = (_iota((256, 512), 0) // 16) == (_iota((256, 512), 1) % 16)
        rsel = _sel(_iota((128, 256), 1) % 16 == _feat(_iota((128, 256), 0)))
        hmask = _head8(_iota((128, 512), 0)) == ((_iota((128, 512), 1) // 16) % 8)
        cp_wphi.wait()
        w2 = wphi_ref[...].reshape(DH * DH, H)
        y = jnp.where(cmask, _dot(w2, eh), 0.0).astype(BF)
        bT = jnp.where(hmask, _dot(rsel, y), 0.0).astype(BF)
        bT_ref[...] = bT
        cp_x(0).wait()
        cp_wk.wait()
        cp_x(1).start()
        ln_tile(0)
        for g in range(NG):
            bg = bT[:, g * 128:(g + 1) * 128]
            w = wqkv_ref[:, 512 + g * 128: 512 + (g + 1) * 128]
            wcatT_ref[512 + g * 128: 512 + (g + 1) * 128, :] = _dot(bg, w, NT).astype(BF)
        cp_wv.wait()
        for i in range(2, NTILE):
            cp_x(i).start()
        for g in range(NG):
            wv = wqkv_ref[:, 1024 + g * 128: 1024 + (g + 1) * 128]
            wcatT_ref[1024 + g * 128: 1024 + (g + 1) * 128, :] = _dot(pmT, wv, NT).astype(BF)

        def kside(i):
            rows = tile_rows(i)
            xnb = xn_ref[rows, :]
            if not isinstance(i, int):
                ln_tile(i + 1)
            pvT = _dot(wcatT_ref[512:1536, :], xnb, NT)
            vTb = pvT[512:1024, :].astype(BF)
            vT_ref[i] = vTb
            ones16 = jnp.ones((16, T), BF)
            for q in range(NQ):
                a, b = _softmax_pair(pvT[q * 64:(q + 1) * 64, :].reshape(8, 8, T))
                phi = jnp.concatenate([a.reshape(64, T), b.reshape(64, T)], axis=0)
                phib = phi.astype(BF)
                phik_ref[i, q * 128:(q + 1) * 128, :] = phi
                phikb_ref[i, q * 128:(q + 1) * 128, :] = phib
                vq = jnp.concatenate([vTb[q * 64:(q + 1) * 64, :], ones16], axis=0)
                kz = _dot(vq, phib, NT)
                kvT_ref[q * 64:(q + 1) * 64, :] = jnp.where(i > 0, kvT_ref[q * 64:(q + 1) * 64, :], 0.0) + kz[0:64]
                z_ref[q * 8:(q + 1) * 8, :] = jnp.where(i > 0, z_ref[q * 8:(q + 1) * 8, :], 0.0) + kz[64:72]

        def phaseA(i, carry):
            cp_x(i + 1).wait()

            @pl.when(i == 1)
            def _():
                cp_wq.start()
                cp_wo.start()
                cp_wg.start()

            @pl.when(i == 2)
            def _():
                cp_wu.start()
                cp_wd.start()

            @pl.when(i == 4)
            def _():
                for j in range(NTILE):
                    cp_dy(j).start()

            kside(i)
            return carry

        lax.fori_loop(0, NTILE - 1, phaseA, 0)

        maskkv = (_iota((512, 128), 0) % 4) == (_iota((512, 128), 1) % 4)

        def finish_kv(accT_ref, zacc_ref, rowform):
            kvmT = jnp.where(maskkv, accT_ref[...], 0.0)
            kvmT_ref[...] = kvmT.astype(BF)
            for q in range(NQ):
                kvm_ref[q * 128:(q + 1) * 128, :] = kvmT[q * 64:(q + 1) * 64, :].T.astype(BF)
            if rowform:
                for q in range(NQ):
                    zrow = zacc_ref[q * 8:q * 8 + 1, :]
                    zb_ref[q * 128:(q + 1) * 128, :] = jnp.broadcast_to(zrow, (128, 128)).T
            else:
                zb_ref[...] = jnp.broadcast_to(jnp.sum(zacc_ref[...], axis=1, keepdims=True), (1024, 128))

        cp_wq.wait()
        cp_wo.wait()
        kside(NTILE - 1)
        for g in range(NG):
            bg = bT_ref[:, g * 128:(g + 1) * 128]
            w = wqkv_ref[:, g * 128:(g + 1) * 128]
            wpT = _dot(bg, w, NT)
            wcat_ref[:, g * 128:(g + 1) * 128] = wpT.T.astype(BF)
            wcatT_ref[g * 128:(g + 1) * 128, :] = wpT.astype(BF)
            wop_ref[g * 128:(g + 1) * 128, :] = _dot(pmT, wo_ref[g * 128:(g + 1) * 128, :]).astype(BF)
        finish_kv(kvT_ref, z_ref, True)
        cp_wg.wait()
        cp_wu.wait()
        cp_wd.wait()

        def phaseB(i, carry):
            rows = tile_rows(i)
            cp_dy(i).wait()
            xnb = xn_ref[rows, :]
            xnT = xnb.astype(F32).T.astype(BF)
            dy = dy_ref[rows, :]
            dyT = dy.astype(F32).T.astype(BF)
            pqT = _dot(wcatT_ref[0:512, :], xnb, NT)
            doT = _dot(wop_ref[...], dy, NT)
            o_parts = []
            dp_parts = []
            g_parts = []
            u_parts = []
            for q in range(NQ):
                a, b = _softmax_pair(pqT[q * 64:(q + 1) * 64, :].reshape(8, 8, T))
                phi = jnp.concatenate([a, b], axis=0)
                phib = phi.reshape(128, T).astype(BF)
                zg = zb_ref[q * 128:(q + 1) * 128, :]
                zg = jnp.concatenate([zg] * (T // 128), axis=1).reshape(16, 8, T)
                den = _hred(phi * zg, jnp.add) + 1e-6
                inv = 1.0 / den
                numT = _dot(kvmT_ref[q * 64:(q + 1) * 64, :], phib)
                oT = numT.reshape(8, 8, T) * inv
                o_parts.append(oT.reshape(64, T).astype(BF))
                do3 = doT[q * 64:(q + 1) * 64, :].reshape(8, 8, T)
                dnum = do3 * inv
                dden = -_hred(do3 * oT, jnp.add) * inv
                dnumb = dnum.reshape(64, T).astype(BF)
                dphi = _dot(kvm_ref[q * 128:(q + 1) * 128, :], dnumb).reshape(16, 8, T) + zg * dden
                dkvTa_ref[q * 64:(q + 1) * 64, :] = (
                    jnp.where(i > 0, dkvTa_ref[q * 64:(q + 1) * 64, :], 0.0) + _dot(dnumb, phib, NT))
                dz_ref[q * 128:(q + 1) * 128, :] = (
                    jnp.where(i > 0, dz_ref[q * 128:(q + 1) * 128, :], 0.0)
                    + _lane_partial((phi * dden).reshape(128, T)))
                dp = _softmax_pair_bwd(a, b, dphi[0:8], dphi[8:16])
                dp_parts.append(dp.reshape(64, T).astype(BF))
                if q < 7:
                    g_parts.append(_dot(xnb, wg_ref[:, q * 256:(q + 1) * 256]))
                    u_parts.append(_dot(xnb, wu_ref[:, q * 256:(q + 1) * 256]))
            oT = jnp.concatenate(o_parts, axis=0)
            dpT = jnp.concatenate(dp_parts, axis=0)

            gg = jnp.concatenate(g_parts, axis=1)
            uu = jnp.concatenate(u_parts, axis=1)
            hb = (gg * uu).astype(BF)
            out_ref[rows, :] = (x_ref[rows, :].astype(F32) + _dot(hb, wd_ref[...])
                                + _dot(oT, wop_ref[...], TN)).astype(BF)
            cp_out(i).start()
            dh = _dot(dy, wd_ref[...], NT)
            dgb = (dh * uu).astype(BF)
            dub = (dh * gg).astype(BF)
            nf = i > 0
            agw = jnp.where(nf, agw_ref[...], 0.0) + _dot(xnT, dgb)
            agw_ref[...] = agw
            dwg_ref[...] = agw.astype(BF)
            auw = jnp.where(nf, auw_ref[...], 0.0) + _dot(xnT, dub)
            auw_ref[...] = auw
            dwu_ref[...] = auw.astype(BF)
            adwT = jnp.where(nf, adwT_ref[...], 0.0) + _dot(dyT, hb)
            adwT_ref[...] = adwT
            dwd_ref[...] = adwT.T.astype(BF)
            dxn_ref[rows, :] = _dot(dgb, wg_ref[...], NT) + _dot(dub, wu_ref[...], NT)

            awo_ref[...] = jnp.where(nf, awo_ref[...], 0.0) + _dot(oT, dy)
            dxnT_ref[i] = _dot(wcat_ref[:, 0:512], dpT)
            gT_ref[0:512, :] = jnp.where(nf, gT_ref[0:512, :], 0.0) + _dot(dpT, xnb)
            return carry

        lax.fori_loop(0, NTILE, phaseB, 0)

        def stage1(i):
            rows = tile_rows(i)
            vTb = vT_ref[i]
            dp_parts = []
            dv_parts = []
            for q in range(NQ):
                phi = phik_ref[i, q * 128:(q + 1) * 128, :].reshape(16, 8, T)
                phib = phikb_ref[i, q * 128:(q + 1) * 128, :]
                zg = zb_ref[q * 128:(q + 1) * 128, :]
                zg = jnp.concatenate([zg] * (T // 128), axis=1)
                dphi = (_dot(kvm_ref[q * 128:(q + 1) * 128, :], vTb[q * 64:(q + 1) * 64, :]) + zg
                        ).reshape(16, 8, T)
                dv_parts.append(_dot(kvmT_ref[q * 64:(q + 1) * 64, :], phib).astype(BF))
                dp = _softmax_pair_bwd(phi[0:8], phi[8:16], dphi[0:8], dphi[8:16])
                dp_parts.append(dp.reshape(64, T).astype(BF))
            dkvT = jnp.concatenate(dp_parts + dv_parts, axis=0)
            dkvT_ref[i] = dkvT
            if isinstance(i, int) and i == 0:
                gT_ref[512:1536, :] = _dot(dkvT, xn_ref[rows, :])
            else:
                gT_ref[512:1536, :] += _dot(dkvT, xn_ref[rows, :])

        def stage2(i):
            rows = tile_rows(i)
            dxnT = dxnT_ref[i] + _dot(wcat_ref[:, 512:1536], dkvT_ref[i])
            dxn = dxn_ref[rows, :] + dxnT.T
            x = x_ref[rows, :].astype(F32)
            xn, r = _layernorm(x)
            m1 = jnp.mean(dxn, axis=-1, keepdims=True)
            m2 = jnp.mean(dxn * xn, axis=-1, keepdims=True)
            dx = dy_ref[rows, :].astype(F32) + r * (dxn - m1 - xn * m2)
            dx_ref[rows, :] = dx.astype(BF)
            cp_dx(i).start()

        cp_dwg.start()
        cp_dwu.start()
        cp_dwd.start()
        finish_kv(dkvTa_ref, dz_ref, False)
        wcat_ref[:, 512:1536] = wcatT_ref[512:1536, :].astype(F32).T.astype(BF)
        stage1(0)
        for g in range(NG):
            dwo_ref[g * 128:(g + 1) * 128, :] = _dot(pm, awo_ref[g * 128:(g + 1) * 128, :].astype(BF)).astype(BF)
        for g in range(NG):
            bg = bT_ref[:, g * 128:(g + 1) * 128]
            gt = gT_ref[g * 128:(g + 1) * 128, :].astype(BF)
            dwqkv_ref[:, g * 128:(g + 1) * 128] = _dot(gt, bg, TN).astype(BF)
            ct_ref[:, g * 128:(g + 1) * 128] = _dot(gt, wqkv_ref[:, g * 128:(g + 1) * 128])
        cp_dwo.start()
        cp_dwq.start()

        def phaseC(i, carry):
            stage2(i - 1)
            stage1(i)
            return carry

        lax.fori_loop(1, NTILE, phaseC, 0)

        gts = []
        for g in range(NG):
            bg = bT_ref[:, g * 128:(g + 1) * 128]
            gt = gT_ref[512 + g * 128: 512 + (g + 1) * 128, :].astype(BF)
            gts.append(gt)
            dwqkv_ref[:, 512 + g * 128: 512 + (g + 1) * 128] = _dot(gt, bg, TN).astype(BF)
            gv = gT_ref[1024 + g * 128: 1024 + (g + 1) * 128, :].astype(BF)
            dwqkv_ref[:, 1024 + g * 128: 1024 + (g + 1) * 128] = _dot(gv, pmT, TN).astype(BF)
        cp_dwkv.start()
        stage2(NTILE - 1)
        cts = []
        for g in range(NG):
            cts.append(ct_ref[:, g * 128:(g + 1) * 128]
                       + _dot(gts[g], wqkv_ref[:, 512 + g * 128: 512 + (g + 1) * 128]))
        ctm = jnp.where(hmask, jnp.concatenate(cts, axis=1), 0.0).astype(BF)
        zz = jnp.where(cmask, _dot(rsel, ctm, TN), 0.0).astype(BF)
        dwphi_ref[...] = _dot(zz, eh, NT).astype(BF).reshape(DH, DH, H)
        cp_dwphi.start()

        pltpu.make_async_copy(out_ref, out_hbm, sem_out.at[0]).wait()
        for c in cp_o:
            c.wait()
        pltpu.make_async_copy(dx_ref, dx_hbm, sem_dx.at[0]).wait()

    scratch = [
        pltpu.VMEM((S, D), BF), pltpu.VMEM((D, 3 * D), BF), pltpu.VMEM((DH, DH, H), BF), pltpu.VMEM((D, D), BF),
        pltpu.VMEM((D, F), BF), pltpu.VMEM((D, F), BF), pltpu.VMEM((F, D), BF), pltpu.VMEM((S, D), BF),
        pltpu.VMEM((S, D), BF), pltpu.VMEM((S, D), BF), pltpu.VMEM((D, 3 * D), BF), pltpu.VMEM((DH, DH, H), BF),
        pltpu.VMEM((D, D), BF), pltpu.VMEM((D, F), BF), pltpu.VMEM((D, F), BF), pltpu.VMEM((F, D), BF),
        pltpu.SemaphoreType.DMA((NTILE,)), pltpu.SemaphoreType.DMA((NTILE,)), pltpu.SemaphoreType.DMA((8,)),
        pltpu.SemaphoreType.DMA((1,)), pltpu.SemaphoreType.DMA((1,)), pltpu.SemaphoreType.DMA((7,)),
        pltpu.VMEM((512, 1536), BF),
        pltpu.VMEM((1536, 512), BF),
        pltpu.VMEM((512, 512), BF),
        pltpu.VMEM((128, 512), BF),
        pltpu.VMEM((S, D), BF),
        pltpu.VMEM((NTILE, 512, T), BF),
        pltpu.VMEM((NTILE, 1024, T), F32),
        pltpu.VMEM((NTILE, 1024, T), BF),
        pltpu.VMEM((S, D), F32),
        pltpu.VMEM((NTILE, 512, T), F32),
        pltpu.VMEM((NTILE, 1024, T), BF),
        pltpu.VMEM((512, 128), F32),
        pltpu.VMEM((64, 128), F32),
        pltpu.VMEM((512, 128), F32),
        pltpu.VMEM((1024, 128), F32),
        pltpu.VMEM((1024, 64), BF),
        pltpu.VMEM((512, 128), BF),
        pltpu.VMEM((1024, 128), F32),
        pltpu.VMEM((512, F), F32),
        pltpu.VMEM((512, F), F32),
        pltpu.VMEM((512, F), F32),
        pltpu.VMEM((1536, 512), F32),
        pltpu.VMEM((512, 512), F32),
        pltpu.VMEM((128, 512), F32),
    ]
    return kernel, scratch


@jax.jit
def pallas_parallel_sum__linear_kernel_hedgehog__glu_gated_bilinear__prompt_kernel(
    A_x: jax.Array,
    A_wqkv: jax.Array,
    A_w_phi: jax.Array,
    A_wo: jax.Array,
    B_x: jax.Array,
    B_w_gate: jax.Array,
    B_w_up: jax.Array,
    B_w_down: jax.Array,
    grad_out: jax.Array,
):
    del B_x
    kernel, scratch = _make_kernel(256)
    out_shape = (
        jax.ShapeDtypeStruct((S, D), BF),
        jax.ShapeDtypeStruct((S, D), BF),
        jax.ShapeDtypeStruct((D, 3 * D), BF),
        jax.ShapeDtypeStruct((DH, DH, H), BF),
        jax.ShapeDtypeStruct((D, D), BF),
        jax.ShapeDtypeStruct((D, F), BF),
        jax.ShapeDtypeStruct((D, F), BF),
        jax.ShapeDtypeStruct((F, D), BF),
    )
    anyspec = pl.BlockSpec(memory_space=pl.ANY)
    outs = pl.pallas_call(
        kernel,
        out_shape=out_shape,
        in_specs=[anyspec] * 8,
        out_specs=[anyspec] * 8,
        scratch_shapes=scratch,
        compiler_params=pltpu.CompilerParams(vmem_limit_bytes=120 * 1024 * 1024),
    )(A_x.reshape(S, D), A_wqkv, jnp.transpose(A_w_phi, (1, 2, 0)), A_wo, B_w_gate, B_w_up, B_w_down,
      grad_out.reshape(S, D))
    out, dx, dwqkv, dwphi, dwo, dwg, dwu, dwd = outs
    return (out.reshape(1, S, D), dx.reshape(1, S, D), dwqkv, jnp.transpose(dwphi, (2, 0, 1)), dwo, dwg, dwu, dwd)
```

```python
import jax
import jax.numpy as jnp
from jax import lax
import jax.experimental.pallas as pl
import jax.experimental.pallas.tpu as pltpu

S, D, H, DH, F = 2048, 512, 32, 16, 1792
NG = 4
NQ = 8
RB = 120
RP = NG * RB
BF = jnp.bfloat16
F32 = jnp.float32

NN = (((1,), (0,)), ((), ()))
NT = (((1,), (1,)), ((), ()))
TN = (((0,), (0,)), ((), ()))


def _dot(a, b, dims=NN):
    return lax.dot_general(a, b, dims, preferred_element_type=F32)


def _iota(shape, dim):
    return lax.broadcasted_iota(jnp.int32, shape, dim)


def _sel(cond):
    return jnp.where(cond, 1.0, 0.0).astype(BF)


def _feat(r):
    return ((r % 64) // 8) * 2 + (r % 8) // 4


def _head8(r):
    return ((r % 128) // 64) * 4 + r % 4


def _rfeat(r):
    return jnp.where(r < 112, ((r % 56) // 8) * 2 + (r % 8) // 4, jnp.where(r < RB, 14, 15))


def _rhead8(r):
    return jnp.where(r < 112, (r // 56) * 4 + r % 4, r % 8)


def _hred(x, op):
    r = x[0]
    for k in range(1, x.shape[0]):
        r = op(r, x[k])
    r = op(r, pltpu.roll(r, 4, 0))
    return r[None]


def _expand_p(pblk, qq):
    T = pblk.shape[-1]
    sh = pblk[112:120, :]
    if qq:
        sh = pltpu.roll(sh, 4, 0)
    last = jnp.where(_iota((8, T), 0) < 4, sh, 0.0)
    return jnp.concatenate([pblk[qq * 56:(qq + 1) * 56, :].reshape(7, 8, T), last[None]], axis=0)


def _reduce_dp(dp0, dp1):
    T = dp0.shape[-1]
    sh = jnp.where(_iota((8, T), 0) < 4, dp0[7], pltpu.roll(dp1[7], 4, 0))
    return jnp.concatenate([dp0[0:7], dp1[0:7], sh[None]], axis=0).reshape(RB, T)


def _softmax_pair(p3):
    mx = _hred(p3, jnp.maximum)
    mn = _hred(p3, jnp.minimum)
    ea = jnp.exp(p3 - mx)
    eb = jnp.exp(mn - p3)
    a = ea * (1.0 / _hred(ea, jnp.add))
    b = eb * (1.0 / _hred(eb, jnp.add))
    return a, b


def _softmax_pair_bwd(a, b, da, db):
    dpa = a * (da - _hred(a * da, jnp.add))
    dpb = b * (db - _hred(b * db, jnp.add))
    return dpa - dpb


def _lane_partial(x):
    T = x.shape[-1]
    acc = x[:, 0:128]
    for j in range(1, T // 128):
        acc = acc + x[:, j * 128:(j + 1) * 128]
    return acc


def _layernorm(x):
    m = jnp.mean(x, axis=-1, keepdims=True)
    xc = x - m
    v = jnp.mean(xc * xc, axis=-1, keepdims=True)
    r = lax.rsqrt(v + 1e-5)
    return xc * r, r


def _make_kernel(T):
    NTILE = S // T

    def kernel(x_hbm, wqkv_hbm, wphi_hbm, wo_hbm, wg_hbm, wu_hbm, wd_hbm, dy_hbm,
               out_hbm, dx_hbm, dwqkv_hbm, dwphi_hbm, dwo_hbm, dwg_hbm, dwu_hbm, dwd_hbm,
               x_ref, wqkv_ref, wphi_ref, wo_ref, wg_ref, wu_ref, wd_ref, dy_ref,
               out_ref, dx_ref, dwqkv_ref, dwphi_ref, dwo_ref, dwg_ref, dwu_ref, dwd_ref,
               sem_x, sem_dy, sem_w, sem_out, sem_dx, sem_dw,
               wq_ref, wqT_ref, wkv_ref, wkvT_ref, wop_ref, bT_ref,
               xn_ref, vT_ref, phik_ref, phikb_ref, dxn_ref, dxnT_ref, dkvT_ref,
               kvT_ref, z_ref, dkvTa_ref, dz_ref,
               kvm_ref, kvmT_ref, zb_ref,
               agw_ref, auw_ref, adwT_ref, gq_ref, gkv_ref, awo_ref, ct_ref):

        def tile_rows(i):
            if isinstance(i, int):
                return pl.ds(i * T, T)
            return pl.ds(pl.multiple_of(i * T, T), T)

        def cp_x(i):
            return pltpu.make_async_copy(x_hbm.at[tile_rows(i)], x_ref.at[tile_rows(i)], sem_x.at[i])

        def cp_dy(i):
            return pltpu.make_async_copy(dy_hbm.at[tile_rows(i)], dy_ref.at[tile_rows(i)], sem_dy.at[i])

        def cp_out(i):
            return pltpu.make_async_copy(out_ref.at[tile_rows(i)], out_hbm.at[tile_rows(i)], sem_out.at[0])

        def cp_dx(i):
            return pltpu.make_async_copy(dx_ref.at[tile_rows(i)], dx_hbm.at[tile_rows(i)], sem_dx.at[0])

        w_in = [(wphi_hbm, wphi_ref), (wqkv_hbm.at[:, 512:1024], wqkv_ref.at[:, 512:1024]),
                (wqkv_hbm.at[:, 0:512], wqkv_ref.at[:, 0:512]),
                (wg_hbm, wg_ref), (wu_hbm, wu_ref), (wd_hbm, wd_ref), (wo_hbm, wo_ref),
                (wqkv_hbm.at[:, 1024:1536], wqkv_ref.at[:, 1024:1536])]
        cp_w = [pltpu.make_async_copy(s, d, sem_w.at[k]) for k, (s, d) in enumerate(w_in)]
        cp_wphi, cp_wk, cp_wq, cp_wg, cp_wu, cp_wd, cp_wo, cp_wv = cp_w
        w_out = [(dwg_ref, dwg_hbm), (dwu_ref, dwu_hbm), (dwd_ref, dwd_hbm), (dwo_ref, dwo_hbm),
                 (dwqkv_ref.at[:, 0:512], dwqkv_hbm.at[:, 0:512]),
                 (dwqkv_ref.at[:, 512:1536], dwqkv_hbm.at[:, 512:1536]),
                 (dwphi_ref, dwphi_hbm)]
        cp_o = [pltpu.make_async_copy(s, d, sem_dw.at[k]) for k, (s, d) in enumerate(w_out)]
        cp_dwg, cp_dwu, cp_dwd, cp_dwo, cp_dwq, cp_dwkv, cp_dwphi = cp_o

        def ln_tile(i):
            rows = tile_rows(i)
            xn, _ = _layernorm(x_ref[rows, :].astype(F32))
            xn_ref[rows, :] = xn.astype(BF)

        def fold_w(bT, col0):
            low = _iota((8, D), 0) < 4
            parts = []
            for g in range(NG):
                p = _dot(bT[:, g * 128:(g + 1) * 128],
                         wqkv_ref[:, col0 + g * 128: col0 + (g + 1) * 128], NT).reshape(16, 8, D)
                ref15 = p[15]
                ref15r = pltpu.roll(ref15, 4, 0)
                parts.append(p[0:7] - jnp.where(low, ref15, ref15r)[None])
                parts.append(p[7:14] - jnp.where(low, ref15r, ref15)[None])
                parts.append(p[14:15] - ref15[None])
            parts.append(jnp.zeros(((D - RP) // 8, 8, D), F32))
            return jnp.concatenate(parts, axis=0).reshape(D, D)

        cp_wphi.start()
        cp_wk.start()
        cp_x(0).start()
        cp_wv.start()

        r128 = _iota((128, 128), 0)
        c128 = _iota((128, 128), 1)
        pm = _sel((r128 // 16 == _head8(c128)) & (r128 % 16 == _feat(c128)))
        pmT = _sel((c128 // 16 == _head8(r128)) & (c128 % 16 == _feat(r128)))
        eh = _sel(_iota((32, 512), 0) == _iota((32, 512), 1) // 16)
        cmask = (_iota((256, 512), 0) // 16) == (_iota((256, 512), 1) % 16)
        rsel = _sel(_iota((128, 256), 1) % 16 == _rfeat(_iota((128, 256), 0)))
        hmask = _rhead8(_iota((128, 512), 0)) == ((_iota((128, 512), 1) // 16) % 8)
        cp_wphi.wait()
        w2 = wphi_ref[...].reshape(DH * DH, H)
        y = jnp.where(cmask, _dot(w2, eh), 0.0).astype(BF)
        bT = jnp.where(hmask, _dot(rsel, y), 0.0).astype(BF)
        bT_ref[...] = bT
        cp_x(0).wait()
        cp_wk.wait()
        cp_x(1).start()
        ln_tile(0)
        wkT = fold_w(bT, 512).astype(BF)
        wkvT_ref[0:RP, :] = wkT[0:RP]
        wkvT_ref[RP + 512:1024, :] = wkT[RP:512]
        cp_wv.wait()
        for i in range(2, NTILE):
            cp_x(i).start()
        for g in range(NG):
            wv = wqkv_ref[:, 1024 + g * 128: 1024 + (g + 1) * 128]
            wkvT_ref[RP + g * 128:RP + (g + 1) * 128, :] = _dot(pmT, wv, NT).astype(BF)

        def kside(i):
            rows = tile_rows(i)
            xnb = xn_ref[rows, :]
            if not isinstance(i, int):
                ln_tile(i + 1)
            pkT = _dot(wkvT_ref[0:RP + 512, :], xnb, NT)
            vTb = pkT[RP:RP + 512, :].astype(BF)
            vT_ref[i] = vTb
            ones16 = jnp.ones((16, T), BF)
            for q in range(NQ):
                a, b = _softmax_pair(_expand_p(pkT[(q // 2) * RB:(q // 2 + 1) * RB, :], q % 2))
                phi = jnp.concatenate([a.reshape(64, T), b.reshape(64, T)], axis=0)
                phib = phi.astype(BF)
                phik_ref[i, q * 128:(q + 1) * 128, :] = phi
                phikb_ref[i, q * 128:(q + 1) * 128, :] = phib
                vq = jnp.concatenate([vTb[q * 64:(q + 1) * 64, :], ones16], axis=0)
                kz = _dot(vq, phib, NT)
                kvT_ref[q * 64:(q + 1) * 64, :] = jnp.where(i > 0, kvT_ref[q * 64:(q + 1) * 64, :], 0.0) + kz[0:64]
                z_ref[q * 8:(q + 1) * 8, :] = jnp.where(i > 0, z_ref[q * 8:(q + 1) * 8, :], 0.0) + kz[64:72]

        def phaseA(i, carry):
            cp_x(i + 1).wait()

            @pl.when(i == 1)
            def _():
                cp_wq.start()
                cp_wo.start()
                cp_wg.start()

            @pl.when(i == 2)
            def _():
                cp_wu.start()
                cp_wd.start()

            @pl.when(i == 4)
            def _():
                for j in range(NTILE):
                    cp_dy(j).start()

            kside(i)
            return carry

        lax.fori_loop(0, NTILE - 1, phaseA, 0)

        maskkv = (_iota((512, 128), 0) % 4) == (_iota((512, 128), 1) % 4)

        def finish_kv(accT_ref, zacc_ref, rowform):
            kvmT = jnp.where(maskkv, accT_ref[...], 0.0)
            kvmT_ref[...] = kvmT.astype(BF)
            for q in range(NQ):
                kvm_ref[q * 128:(q + 1) * 128, :] = kvmT[q * 64:(q + 1) * 64, :].T.astype(BF)
            if rowform:
                for q in range(NQ):
                    zrow = zacc_ref[q * 8:q * 8 + 1, :]
                    zb_ref[q * 128:(q + 1) * 128, :] = jnp.broadcast_to(zrow, (128, 128)).T
            else:
                zb_ref[...] = jnp.broadcast_to(jnp.sum(zacc_ref[...], axis=1, keepdims=True), (1024, 128))

        cp_wq.wait()
        cp_wo.wait()
        kside(NTILE - 1)
        wqT = fold_w(bT_ref[...], 0)
        wqT_ref[...] = wqT.astype(BF)
        wq_ref[...] = wqT.T.astype(BF)
        for g in range(NG):
            wop_ref[g * 128:(g + 1) * 128, :] = _dot(pmT, wo_ref[g * 128:(g + 1) * 128, :]).astype(BF)
        finish_kv(kvT_ref, z_ref, True)
        cp_wg.wait()
        cp_wu.wait()
        cp_wd.wait()

        def phaseB(i, carry):
            rows = tile_rows(i)
            cp_dy(i).wait()
            xnb = xn_ref[rows, :]
            xnT = xnb.astype(F32).T.astype(BF)
            dy = dy_ref[rows, :]
            dyT = dy.astype(F32).T.astype(BF)
            g_parts = [_dot(xnb, wg_ref[:, 0:256])]
            u_parts = []
            pqT = _dot(wqT_ref[0:RP, :], xnb, NT)
            doT = _dot(wop_ref[...], dy, NT)
            o_parts = []
            dp_parts = []
            dh_parts = []
            for q in range(NQ):
                if q < 6:
                    g_parts.append(_dot(xnb, wg_ref[:, (q + 1) * 256:(q + 2) * 256]))
                a, b = _softmax_pair(_expand_p(pqT[(q // 2) * RB:(q // 2 + 1) * RB, :], q % 2))
                phi = jnp.concatenate([a, b], axis=0)
                phib = phi.reshape(128, T).astype(BF)
                zg = zb_ref[q * 128:(q + 1) * 128, :]
                zg = jnp.concatenate([zg] * (T // 128), axis=1).reshape(16, 8, T)
                den = _hred(phi * zg, jnp.add) + 1e-6
                inv = 1.0 / den
                numT = _dot(kvmT_ref[q * 64:(q + 1) * 64, :], phib)
                oT = numT.reshape(8, 8, T) * inv
                o_parts.append(oT.reshape(64, T).astype(BF))
                if q >= 1:
                    dh_parts.append(_dot(dy, wd_ref[(q - 1) * 256:q * 256, :], NT))
                do3 = doT[q * 64:(q + 1) * 64, :].reshape(8, 8, T)
                dnum = do3 * inv
                dden = -_hred(do3 * oT, jnp.add) * inv
                dnumb = dnum.reshape(64, T).astype(BF)
                dphi = _dot(kvm_ref[q * 128:(q + 1) * 128, :], dnumb).reshape(16, 8, T) + zg * dden
                dkvTa_ref[q * 64:(q + 1) * 64, :] = (
                    jnp.where(i > 0, dkvTa_ref[q * 64:(q + 1) * 64, :], 0.0) + _dot(dnumb, phib, NT))
                dz_ref[q * 128:(q + 1) * 128, :] = (
                    jnp.where(i > 0, dz_ref[q * 128:(q + 1) * 128, :], 0.0)
                    + _lane_partial((phi * dden).reshape(128, T)))
                if q < 7:
                    u_parts.append(_dot(xnb, wu_ref[:, q * 256:(q + 1) * 256]))
                dp_parts.append(_softmax_pair_bwd(a, b, dphi[0:8], dphi[8:16]))
            oT = jnp.concatenate(o_parts, axis=0)
            dpT = jnp.concatenate(
                [_reduce_dp(dp_parts[2 * g], dp_parts[2 * g + 1]) for g in range(NG)]
                + [jnp.zeros((D - RP, T), F32)], axis=0).astype(BF)

            gg = jnp.concatenate(g_parts, axis=1)
            uu = jnp.concatenate(u_parts, axis=1)
            hb = (gg * uu).astype(BF)
            out_ref[rows, :] = (x_ref[rows, :].astype(F32) + _dot(hb, wd_ref[...])
                                + _dot(oT, wop_ref[...], TN)).astype(BF)
            cp_out(i).start()
            dh = jnp.concatenate(dh_parts, axis=1)
            dgb = (dh * uu).astype(BF)
            dub = (dh * gg).astype(BF)
            nf = i > 0
            agw = jnp.where(nf, agw_ref[...], 0.0) + _dot(xnT, dgb)
            agw_ref[...] = agw
            dwg_ref[...] = agw.astype(BF)
            auw = jnp.where(nf, auw_ref[...], 0.0) + _dot(xnT, dub)
            auw_ref[...] = auw
            dwu_ref[...] = auw.astype(BF)
            adwT = jnp.where(nf, adwT_ref[...], 0.0) + _dot(dyT, hb)
            adwT_ref[...] = adwT
            dwd_ref[...] = adwT.T.astype(BF)
            dxn_ref[rows, :] = _dot(dgb, wg_ref[...], NT) + _dot(dub, wu_ref[...], NT)

            awo_ref[...] = jnp.where(nf, awo_ref[...], 0.0) + _dot(oT, dy)
            dxnT_ref[i] = _dot(wq_ref[...], dpT)
            gq_ref[...] = jnp.where(nf, gq_ref[...], 0.0) + _dot(dpT[0:RP], xnb)
            return carry

        lax.fori_loop(0, NTILE, phaseB, 0)

        def stage1(i):
            rows = tile_rows(i)
            vTb = vT_ref[i]
            dp_parts = []
            dv_parts = []
            for q in range(NQ):
                phi = phik_ref[i, q * 128:(q + 1) * 128, :].reshape(16, 8, T)
                phib = phikb_ref[i, q * 128:(q + 1) * 128, :]
                zg = zb_ref[q * 128:(q + 1) * 128, :]
                zg = jnp.concatenate([zg] * (T // 128), axis=1)
                dphi = (_dot(kvm_ref[q * 128:(q + 1) * 128, :], vTb[q * 64:(q + 1) * 64, :]) + zg
                        ).reshape(16, 8, T)
                dv_parts.append(_dot(kvmT_ref[q * 64:(q + 1) * 64, :], phib).astype(BF))
                dp_parts.append(_softmax_pair_bwd(phi[0:8], phi[8:16], dphi[0:8], dphi[8:16]))
            dpT = jnp.concatenate(
                [_reduce_dp(dp_parts[2 * g], dp_parts[2 * g + 1]) for g in range(NG)], axis=0).astype(BF)
            dkvT = jnp.concatenate([dpT] + dv_parts + [jnp.zeros((D - RP, T), BF)], axis=0)
            dkvT_ref[i] = dkvT
            if isinstance(i, int) and i == 0:
                gkv_ref[...] = _dot(dkvT[0:512 + RP], xn_ref[rows, :])
            else:
                gkv_ref[...] += _dot(dkvT[0:512 + RP], xn_ref[rows, :])

        def stage2(i):
            rows = tile_rows(i)
            dxnT = dxnT_ref[i] + _dot(wkv_ref[...], dkvT_ref[i])
            dxn = dxn_ref[rows, :] + dxnT.T
            x = x_ref[rows, :].astype(F32)
            xn, r = _layernorm(x)
            m1 = jnp.mean(dxn, axis=-1, keepdims=True)
            m2 = jnp.mean(dxn * xn, axis=-1, keepdims=True)
            dx = dy_ref[rows, :].astype(F32) + r * (dxn - m1 - xn * m2)
            dx_ref[rows, :] = dx.astype(BF)
            cp_dx(i).start()

        def g_block(ref, row0, g):
            blk = ref[row0 + g * RB: row0 + (g + 1) * RB, :].reshape(15, 8, D)
            s0 = _hred(blk[0:7], jnp.add)[0]
            s1 = _hred(blk[7:14], jnp.add)[0]
            g15 = -(jnp.where(_iota((8, D), 0) < 4, s0, s1) + blk[14])
            return jnp.concatenate([blk, g15[None]], axis=0).reshape(128, D).astype(BF)

        cp_dwg.start()
        cp_dwu.start()
        cp_dwd.start()
        finish_kv(dkvTa_ref, dz_ref, False)
        wkv_ref[...] = wkvT_ref[...].astype(F32).T.astype(BF)
        stage1(0)
        for g in range(NG):
            dwo_ref[g * 128:(g + 1) * 128, :] = _dot(pm, awo_ref[g * 128:(g + 1) * 128, :].astype(BF)).astype(BF)
        for g in range(NG):
            bg = bT_ref[:, g * 128:(g + 1) * 128]
            gt = g_block(gq_ref, 0, g)
            dwqkv_ref[:, g * 128:(g + 1) * 128] = _dot(gt, bg, TN).astype(BF)
            ct_ref[:, g * 128:(g + 1) * 128] = _dot(gt, wqkv_ref[:, g * 128:(g + 1) * 128])
        cp_dwo.start()
        cp_dwq.start()

        def phaseC(i, carry):
            stage2(i - 1)
            stage1(i)
            return carry

        lax.fori_loop(1, NTILE, phaseC, 0)

        gts = []
        for g in range(NG):
            bg = bT_ref[:, g * 128:(g + 1) * 128]
            gt = g_block(gkv_ref, 0, g)
            gts.append(gt)
            dwqkv_ref[:, 512 + g * 128: 512 + (g + 1) * 128] = _dot(gt, bg, TN).astype(BF)
            gv = gkv_ref[RP + g * 128:RP + (g + 1) * 128, :].astype(BF)
            dwqkv_ref[:, 1024 + g * 128: 1024 + (g + 1) * 128] = _dot(gv, pmT, TN).astype(BF)
        cp_dwkv.start()
        stage2(NTILE - 1)
        cts = []
        for g in range(NG):
            cts.append(ct_ref[:, g * 128:(g + 1) * 128]
                       + _dot(gts[g], wqkv_ref[:, 512 + g * 128: 512 + (g + 1) * 128]))
        ctm = jnp.where(hmask, jnp.concatenate(cts, axis=1), 0.0).astype(BF)
        zz = jnp.where(cmask, _dot(rsel, ctm, TN), 0.0).astype(BF)
        dwphi_ref[...] = _dot(zz, eh, NT).astype(BF).reshape(DH, DH, H)
        cp_dwphi.start()

        pltpu.make_async_copy(out_ref, out_hbm, sem_out.at[0]).wait()
        for c in cp_o:
            c.wait()
        pltpu.make_async_copy(dx_ref, dx_hbm, sem_dx.at[0]).wait()

    scratch = [
        pltpu.VMEM((S, D), BF), pltpu.VMEM((D, 3 * D), BF), pltpu.VMEM((DH, DH, H), BF), pltpu.VMEM((D, D), BF),
        pltpu.VMEM((D, F), BF), pltpu.VMEM((D, F), BF), pltpu.VMEM((F, D), BF), pltpu.VMEM((S, D), BF),
        pltpu.VMEM((S, D), BF), pltpu.VMEM((S, D), BF), pltpu.VMEM((D, 3 * D), BF), pltpu.VMEM((DH, DH, H), BF),
        pltpu.VMEM((D, D), BF), pltpu.VMEM((D, F), BF), pltpu.VMEM((D, F), BF), pltpu.VMEM((F, D), BF),
        pltpu.SemaphoreType.DMA((NTILE,)), pltpu.SemaphoreType.DMA((NTILE,)), pltpu.SemaphoreType.DMA((8,)),
        pltpu.SemaphoreType.DMA((1,)), pltpu.SemaphoreType.DMA((1,)), pltpu.SemaphoreType.DMA((7,)),
        pltpu.VMEM((512, 512), BF),
        pltpu.VMEM((512, 512), BF),
        pltpu.VMEM((512, 1024), BF),
        pltpu.VMEM((1024, 512), BF),
        pltpu.VMEM((512, 512), BF),
        pltpu.VMEM((128, 512), BF),
        pltpu.VMEM((S, D), BF),
        pltpu.VMEM((NTILE, 512, T), BF),
        pltpu.VMEM((NTILE, 1024, T), F32),
        pltpu.VMEM((NTILE, 1024, T), BF),
        pltpu.VMEM((S, D), F32),
        pltpu.VMEM((NTILE, 512, T), F32),
        pltpu.VMEM((NTILE, 1024, T), BF),
        pltpu.VMEM((512, 128), F32),
        pltpu.VMEM((64, 128), F32),
        pltpu.VMEM((512, 128), F32),
        pltpu.VMEM((1024, 128), F32),
        pltpu.VMEM((1024, 64), BF),
        pltpu.VMEM((512, 128), BF),
        pltpu.VMEM((1024, 128), F32),
        pltpu.VMEM((512, F), F32),
        pltpu.VMEM((512, F), F32),
        pltpu.VMEM((512, F), F32),
        pltpu.VMEM((RP, 512), F32),
        pltpu.VMEM((512 + RP, 512), F32),
        pltpu.VMEM((512, 512), F32),
        pltpu.VMEM((128, 512), F32),
    ]
    return kernel, scratch


@jax.jit
def pallas_parallel_sum__linear_kernel_hedgehog__glu_gated_bilinear__prompt_kernel(
    A_x: jax.Array,
    A_wqkv: jax.Array,
    A_w_phi: jax.Array,
    A_wo: jax.Array,
    B_x: jax.Array,
    B_w_gate: jax.Array,
    B_w_up: jax.Array,
    B_w_down: jax.Array,
    grad_out: jax.Array,
):
    del B_x
    kernel, scratch = _make_kernel(256)
    out_shape = (
        jax.ShapeDtypeStruct((S, D), BF),
        jax.ShapeDtypeStruct((S, D), BF),
        jax.ShapeDtypeStruct((D, 3 * D), BF),
        jax.ShapeDtypeStruct((DH, DH, H), BF),
        jax.ShapeDtypeStruct((D, D), BF),
        jax.ShapeDtypeStruct((D, F), BF),
        jax.ShapeDtypeStruct((D, F), BF),
        jax.ShapeDtypeStruct((F, D), BF),
    )
    anyspec = pl.BlockSpec(memory_space=pl.ANY)
    outs = pl.pallas_call(
        kernel,
        out_shape=out_shape,
        in_specs=[anyspec] * 8,
        out_specs=[anyspec] * 8,
        scratch_shapes=scratch,
        compiler_params=pltpu.CompilerParams(vmem_limit_bytes=120 * 1024 * 1024),
    )(A_x.reshape(S, D), A_wqkv, jnp.transpose(A_w_phi, (1, 2, 0)), A_wo, B_w_gate, B_w_up, B_w_down,
      grad_out.reshape(S, D))
    out, dx, dwqkv, dwphi, dwo, dwg, dwu, dwd = outs
    return (out.reshape(1, S, D), dx.reshape(1, S, D), dwqkv, jnp.transpose(dwphi, (2, 0, 1)), dwo, dwg, dwu, dwd)
```
